```python
import jax
import jax.numpy as jnp

def _softmax(x, axis=-1):
    return jax.nn.softmax(x, axis=axis)
def _gelu(x):
    return jax.nn.gelu(x, approximate=True)
def _silu(x):
    return jax.nn.silu(x)
def _sigmoid(x):
    return jax.nn.sigmoid(x)
def _layernorm(x, axis=-1, eps=1e-5):
    m = jnp.mean(x, axis=axis, keepdims=True)
    v = jnp.var(x, axis=axis, keepdims=True)
    return (x - m) / jnp.sqrt(v + eps)
def _scatter_add(tgt, idx, src, axis=0):
    return tgt.at[idx].add(src)
def _segment_sum(src, seg, n):
    return jax.ops.segment_sum(src, seg, n)
class _Rng:
    def __init__(self, key):
        self._k = key
    def _next(self):
        self._k, sub = jax.random.split(self._k)
        return sub
    def normal(self, shape):
        return jax.random.normal(self._next(), shape, dtype=jnp.bfloat16)
    def randint(self, lo, hi, shape):
        return jax.random.randint(self._next(), shape, lo, hi, dtype=jnp.int32)
    def uniform(self, shape, lo=0.0, hi=1.0):
        return jax.random.uniform(self._next(), shape, jnp.bfloat16, lo, hi)
    def permutation(self, n):
        return jax.random.permutation(self._next(), n)


kernel_name = 'sequential_preLN__ssm_conv_s4__moe_arch_mod__prompt'

def setup_inputs():
    _rng = _Rng(jax.random.key(int.from_bytes(__import__("os").urandom(4), "little")))
    _w = (lambda a: (lambda t: t.astype(jnp.bfloat16) if jnp.issubdtype(t.dtype, jnp.floating) else t)(jnp.asarray(a)))
    def _A_setup():
        B, L, D, N = 1, 2048, 576, 128
        A_re = -jnp.exp((lambda *s: _rng.normal(s) * 0.05)(D, N))
        A_im = jnp.pi * (lambda *s: _rng.normal(s) * 0.05)(D, N)
        B_re = (lambda *s: _rng.normal(s) * 0.05)(D, N)
        B_im = (lambda *s: _rng.normal(s) * 0.05)(D, N)
        C_re = (lambda *s: _rng.normal(s) * 0.05)(D, N)
        C_im = (lambda *s: _rng.normal(s) * 0.05)(D, N)
        log_dt = (lambda *s: _rng.normal(s) * 0.05)(D) * 0.5 - 4.0
        Dskip = (lambda *s: _rng.normal(s) * 0.05)(D)
        return {
            "u": _w((lambda *s: _rng.normal(s) * 0.05)(B, L, D)),
            "A_re": _w(A_re),
            "A_im": _w(A_im),
            "B_re": _w(B_re),
            "B_im": _w(B_im),
            "C_re": _w(C_re),
            "C_im": _w(C_im),
            "log_dt": _w(log_dt),
            "Dskip": _w(Dskip),
        }
    _A_in = _A_setup()

    def _B_setup():
        B, S, D, F, C = 1, 2048, 576, 4608, 8
        return {
            "x": _w((lambda *s: _rng.normal(s) * 0.05)(B, S, D)),
            "w_r": _w((lambda *s: _rng.normal(s) * 0.05)(D)),
            "w_gate": _w((lambda *s: _rng.normal(s) * 0.05)(D, F)),
            "w_up": _w((lambda *s: _rng.normal(s) * 0.05)(D, F)),
            "w_down": _w((lambda *s: _rng.normal(s) * 0.05)(F, D)),
        }
    _B_in = _B_setup()

    return {
        "A_u": _A_in["u"],
        "A_A_re": _A_in["A_re"],
        "A_A_im": _A_in["A_im"],
        "A_B_re": _A_in["B_re"],
        "A_B_im": _A_in["B_im"],
        "A_C_re": _A_in["C_re"],
        "A_C_im": _A_in["C_im"],
        "A_log_dt": _A_in["log_dt"],
        "A_Dskip": _A_in["Dskip"],
        "B_x": _B_in["x"],
        "B_w_r": _B_in["w_r"],
        "B_w_gate": _B_in["w_gate"],
        "B_w_up": _B_in["w_up"],
        "B_w_down": _B_in["w_down"],
    }

def reference(A_u, A_A_re, A_A_im, A_B_re, A_B_im, A_C_re, A_C_im, A_log_dt, A_Dskip, B_x, B_w_r, B_w_gate, B_w_up, B_w_down):
    def _A_ref(u, A_re, A_im, B_re, B_im, C_re, C_im, log_dt, Dskip):
        Bsz, L, D = u.shape
        dt = jnp.exp(log_dt)[:, None]
        A = A_re + 1j * A_im
        Bc = B_re + 1j * B_im
        Cc = C_re + 1j * C_im
        logdA = dt * A
        dB = dt * Bc
        l = (lambda x, dt: x.astype(dt))(jnp.arange(L), A_re.dtype)
        P = jnp.exp(logdA[:, :, None] * l[None, None, :])
        K = jnp.einsum("dn,dnl,dn->dl", Cc, P, dB).real
        L2 = 2 * L
        Kp = jnp.pad(K, ((0, 0), (0, L)))
        up = (lambda x, *d: x.transpose(*d))(u, 0, 2, 1)
        up = jnp.pad(up, ((0, 0), (0, 0), (0, L)))
        Kf = (lambda x, axes=(-2,-1): jnp.fft.rfft2(x.astype(jnp.float32), axes=axes))(Kp[:, None, :], axes=(-2, -1))
        Uf = (lambda x, axes=(-2,-1): jnp.fft.rfft2(x.astype(jnp.float32), axes=axes))(up[:, :, None, :], axes=(-2, -1))
        Yf = Uf * Kf[None, :, :, :]
        y = (lambda x, s, axes=(-2,-1): jnp.fft.irfft2(x, s=s, axes=axes).astype(jnp.bfloat16))(Yf, (1, L2), axes=(-2, -1))[:, :, 0, :L]
        y = (lambda x, *d: x.transpose(*d))(y, 0, 2, 1) + u * Dskip[None, None, :]
        return y

    def _B_ref(x, w_r, w_gate, w_up, w_down):
        B, S, D = x.shape
        C = 8
        r = x @ w_r
        idx = jnp.argsort(-r, axis=-1)[:, :C]
        idx_e = jnp.repeat(idx.reshape(B, C, 1), D, axis=2)
        x_sel = jnp.take_along_axis(x, idx_e, axis=1)
        g = _silu(x_sel @ w_gate)
        u = x_sel @ w_up
        y = (g * u) @ w_down
        r_sel = _sigmoid(jnp.take_along_axis(r, idx, axis=1))
        y = y * r_sel.reshape(B, C, 1)
        b_off = (jnp.arange(B) * S).reshape(B, 1)
        flat_idx = (idx + b_off).reshape(B * C)
        zero = (x * 0.0).reshape(B * S, D)
        upd = _scatter_add(zero, flat_idx, y.reshape(B * C, D), axis=0)
        return x + upd.reshape(B, S, D)

    x = A_u
    h = x + _A_ref(_layernorm(x, axis=-1), A_A_re, A_A_im, A_B_re, A_B_im, A_C_re, A_C_im, A_log_dt, A_Dskip)
    h2 = h + _B_ref(_layernorm(h, axis=-1), B_w_r, B_w_gate, B_w_up, B_w_down)
    return h2
```

```python
import jax
import jax.numpy as jnp
from jax import lax
import jax.experimental.pallas as pl
import jax.experimental.pallas.tpu as pltpu

D = 576
L = 2048
N = 128
F = 4608
CAP = 8
EPS = 1e-5

NT = L // 128
NG = D // 8

HS = 580
PS = 577
SS = 65
ZS = 36

RING = 4
LAG_A, LAG_B, LAG_C, LAG_K, LAG_D = 0, 16, 24, 42, 48
Q_LAG = 4
N_T = 72
PARTS = (0, 5, 14, 36)
SU = 3
PB = 16
PU = 6
XW = 3
XP = 1024
NP = 4
TIE = (150, 500)
DO = (512, 128, 384, 0, 256)
TR = (0, 0, 8, 8, 8, 12, 12, 12, 12)
WT = (1, 2, 3, 4, 5)
WG = 1
SD = (3, 3, 3, 3, 3, 3, 4, 5)
CUTS = (0, 9, 18, 19)
FW = 512

f32 = jnp.float32
bf16 = jnp.bfloat16
i32 = jnp.int32
NT_DIMS = (((1,), (1,)), ((), ()))


def _rnd(x):
    return x.astype(bf16).astype(f32)


def _cmul(ar, ai, br, bi):
    return ar * br - ai * bi, ar * bi + ai * br


def _csq(ar, ai):
    t = ar * ai
    return ar * ar - ai * ai, t + t


def _csqrt(wr, wi):
    big = jnp.clip(jnp.maximum(jnp.abs(wr), jnp.abs(wi)), 2.0 ** -125, 2.0 ** 125)
    e = jnp.log2(big)
    down = jnp.exp2(-e)
    xr, xi = wr * down, wi * down
    p = jnp.exp2(0.5 * jnp.log2(xr * xr + xi * xi)) + jnp.abs(xr)
    q = jnp.exp2(0.5 * ((e - 1.0) - jnp.log2(jnp.maximum(p, 2.0 ** -60))))
    t, o = p * q, xi * q
    pos = xr >= 0
    return jnp.where(pos, t, o), jnp.where(pos, o, t)


def _unpack2(w):
    return pltpu.bitcast(w << 16, f32), pltpu.bitcast(w & (-65536), f32)


def _interleave(a, b):
    return jnp.concatenate([a, b], axis=1).astype(bf16).reshape(2 * a.shape[0], 128)


def _pack2(a, b):
    return pltpu.bitcast(_interleave(a, b), i32)


def _ln_stats(s1, s2):
    m = s1 * (1.0 / D)
    v = _rnd(jnp.maximum(s2 * (1.0 / D) - m * m, 0.0))
    return _rnd(m), 1.0 / _rnd(jnp.sqrt(_rnd(v + _rnd(jnp.full_like(v, EPS)))))


def _span(start, size, align):
    return pl.ds(start if isinstance(start, int) else pl.multiple_of(start, align), size)


def _lanes(c, n=1):
    return _span(128 * n * c, 128 * n, 128 * n)


def _row(ref, k, r, rows):
    return jnp.broadcast_to(ref[k, pl.ds(r, 1), :], (rows, 128))


def _iota(shape, axis):
    return lax.broadcasted_iota(i32, shape, axis)


def _kernel(
    x_hbm, are_hbm, aim_hbm, bre_hbm, bim_hbm, cre_hbm, cim_hbm,
    ldt_hbm, dsk_hbm, wr_hbm, wg_hbm, wu_hbm, wd_hbm,
    o_hbm,
    ldt, dsk, wrt, prm, col, pr, pi, mul, vec, xb, xs, st1, un, ur,
    vs, ss, zs, ys, rs, hs, st2, ob, lb, nb, wg, wu, wd,
    sem_p, sem_o,
):
    def p_cp(j):
        rows = pl.ds(16 * PARTS[j], 16 * (PARTS[j + 1] - PARTS[j]))
        return [pltpu.make_async_copy(src.at[rows], prm.at[k, rows], sem_p.at[1 + j])
                for k, src in enumerate((are_hbm, aim_hbm, bre_hbm, bim_hbm, cre_hbm, cim_hbm))]

    def copy(src, dst, sem, rows=slice(None), cols=slice(None)):
        return pltpu.make_async_copy(src.at[rows, cols], dst.at[rows, cols], sem_p.at[sem])

    def fetch(src, dst, sem, i, c0, width, after):
        rows = _span(8 * i, 8, 8)
        dst[rows, pl.ds(c0, 128)] = after.astype(bf16)
        copy(src, dst, sem, rows, pl.ds(c0, width)).start()

    v_cp = [pltpu.make_async_copy(a, b, sem_p.at[0])
            for a, b in ((ldt_hbm, ldt), (dsk_hbm, dsk), (wr_hbm, wrt))]
    x_cp = [copy(x_hbm, xb, 4, cols=pl.ds(0, 256 * XW)),
            copy(x_hbm, xb, 5, cols=pl.ds(256 * XW, L - 256 * XW))]
    w_cp = [copy(wg_hbm, wg, 6), copy(wu_hbm, wu, 7),
            copy(wd_hbm, wd, 8, pl.ds(0, 256)), copy(wd_hbm, wd, 9, pl.ds(256, D - 256))]
    for c in v_cp + sum([p_cp(j) for j in range(len(PARTS) - 1)], []) + [
            x_cp[0], copy(x_hbm, xb, 5, cols=pl.ds(256 * XW, L - 256 * XW - XP)),
            copy(wg_hbm, wg, 6, pl.ds(112, D - 112)), w_cp[2],
            copy(wd_hbm, wd, 9, pl.ds(256, D - 256 - 8 * NP))]:
        c.start(priority=1)

    lane8, sub8 = _iota((8, 128), 1), _iota((8, 128), 0)

    def lane_sum(v):
        return jnp.broadcast_to(jnp.sum(v, axis=1, keepdims=True), (8, 128))

    for c in v_cp:
        c.wait()
    for k, ref in enumerate((ldt, dsk, wrt)):
        row = ref[...].astype(f32).reshape(1, D)
        row = jnp.concatenate([row, jnp.zeros((1, 640 - D), f32)], axis=1)
        for t in range(5):
            v = jnp.broadcast_to(row[:, 128 * t:128 * t + 128], (8, 128))
            vec[k, t] = v if k else _rnd(jnp.exp(v))

    zero = jnp.minimum(pltpu.bitcast(vec[1, 0], i32)[0, 0] & 1, 0)
    never = (lane8 < zero, sub8 < zero)

    def block(fn):
        pl.loop(0, 1 + zero)(lambda _: fn())

    def powers(q, carry):
        trig, done = carry
        both = [prm[k, _span(16 * q, 16, 16), :].astype(f32) for k in range(6)]
        for e in range(2):
            r0 = pl.multiple_of(16 * q + 8 * e, 8)
            rows = pl.ds(r0, 8)
            own = lane8 - sub8 == (r0 & 127)
            dt, skip, route = [jnp.where(own, vec[k, q >> 3], 0.0) for k in range(3)]
            dt = jnp.where(never[0], done[0], jnp.where(never[1], trig[0], lane_sum(dt)))
            ar, ai, br, bi, cr, ci = [v[8 * e:8 * e + 8] for v in both]
            mag, cos, sin = jnp.exp(dt * ar), jnp.cos(dt * ai), jnp.sin(dt * ai)
            a = mag * cos, mag * sin
            mul[4, rows, :], mul[5, rows, :] = a
            fetch(x_hbm, xb, 5, 2 * q + e, L - XP, XP, mag)
            w = _cmul(cr, ci, dt * br, dt * bi)
            col[0, rows, :], col[1, rows, :] = lane_sum(w[0] + skip), lane_sum(route)
            v = _csqrt(*_cmul(*w, *a))
            a = _csq(*a)
            for j in range(8):
                pr[pl.ds(j * PS + r0, 8), :], pi[pl.ds(j * PS + r0, 8), :] = v
                last, v = v[0], _cmul(*v, *a)
            for _ in range(3):
                a = _csq(*a)
            mul[0, rows, :], mul[1, rows, :] = a
            mul[2, rows, :], mul[3, rows, :] = _csq(*_csq(*a))
            trig, done = trig[1:] + [cos], done[1:] + [last]
        return trig, done

    for j, (lo, hi) in enumerate(zip(PARTS, PARTS[1:])):
        for c in p_cp(j):
            c.wait()
        lax.fori_loop(lo, hi, powers, tuple([jnp.zeros((8, 128), f32)] * k for k in (SU, PU)),
                      unroll=hi - lo)

    def moments(i):
        sums = []
        for c in (2 * i, 2 * i + 1):
            s1, s2 = [None, None], [None, None]
            for q in range(D // 16):
                w = pltpu.bitcast(xb[pl.ds(16 * q, 16), _lanes(c)], i32)
                for e, v in enumerate(_unpack2(w)):
                    xs[pl.ds(c * HS + e * (D // 2) + 8 * q, 8), :] = v
                    s1[e], s2[e] = (s1[e] + v, s2[e] + v * v) if q else (v, v * v)
            fetch(wg_hbm, wg, 6, i, F // 3 * len(sums), F // 3, v)
            sums.append([jnp.sum(v[0] + v[1], axis=0, keepdims=True) for v in (s1, s2)])
        st1[0, i], st1[1, i] = _ln_stats(*[jnp.where(sub8 == 0, u, v) for u, v in zip(*sums)])

    flip = jnp.where(_iota((128, 128), 0) == _iota((128, 128), 1) ^ 63, 1.0, 0.0).astype(bf16)

    def normalise(i):
        m, s = [[_row(st1.at[n], i, e, 8) for e in range(2)] for n in range(2)]
        for q in range(D // 16):
            xa, xc = [[xs[pl.ds(c * HS + e * (D // 2) + 8 * q, 8), :] for e in range(2)]
                      for c in (2 * i, 2 * i + 1)]
            u = [((xa[e] - m[0]) * s[0], (xc[e] - m[1]) * s[1]) for e in range(2)]
            w = [_pack2(*v) for v in u]
            if q % 3 == 0:
                r = jnp.dot(jnp.concatenate(u[0] + u[1], axis=0).astype(bf16), flip,
                            preferred_element_type=f32)
                r = [_pack2(r[n:n + 8], r[n + 8:n + 16]) for n in (0, 16)]
            else:
                r = [jnp.take_along_axis(v, lane8 ^ 63, axis=1, mode="promise_in_bounds")
                     for v in w]
            for e in range(2):
                rows = pl.ds(i * HS + e * (D // 2) + 8 * q, 8)
                un[rows, :], ur[rows, :] = w[e], r[e]
        fetch(wg_hbm, wg, 6, i, F // 3 * 2, F // 3, u[0][0])

    vec[2, 0] = lane_sum(sum(vec[2, t] for t in range(5)))

    @pl.loop(0, 1 + zero)
    def _(_):
        for c, lo, hi in zip(x_cp, (0, XW), (XW, NT // 2)):
            c.wait()
            pl.loop(lo, hi, unroll=hi - lo)(moments)
            pl.loop(max(lo - 1, 0), hi - 1, unroll=hi - 1 - max(lo - 1, 0))(normalise)
        normalise(NT // 2 - 1)

    left8, right8 = lane8 < 64, lane8 >= 64
    left16 = _iota((16, 128), 1) < 64
    lane32, row32 = _iota((32, 128), 1), 2 * _iota((32, 128), 0)
    tri0, tri1 = (lane32 >= row32) & (lane32 < 64), lane32 >= row32 + 64

    def v_tile(r, k):
        return pltpu.bitcast(vs[r, pl.ds(64 * k, 64), :], bf16)

    def channel(ref, g, k, n):
        return ref[pl.ds((k % 2) * (D // 2) + g * 4 + k // 2, n, stride=HS), :]

    def vandermonde(g, r, k):
        ch = g * 8 + k
        vr, vi = pr[pl.ds(ch, 8, stride=PS), :], pi[pl.ds(ch, 8, stride=PS), :]
        odd = _cmul(vr, vi, _row(mul, 4, ch, 8), _row(mul, 5, ch, 8))
        vr, vi = jnp.concatenate([vr, odd[0]], axis=0), jnp.concatenate([vi, odd[1]], axis=0)
        mr, mi = _row(mul, 0, ch, 16), _row(mul, 1, ch, 16)
        re, im = [], []
        for q in range(4):
            re.append(_pack2(vr[:8], vr[8:]))
            im.append(_pack2(vi[:8], vi[8:]))
            vr, vi = _cmul(vr, vi, mr, mi)
        for q, v in enumerate(re + im):
            vs[r, pl.ds(64 * k + 8 * q, 8), :] = v
        return odd[0]

    def chunk_states(g, r, k):
        p1 = channel(ur, g, k, NT // 2)
        p2 = pltpu.roll(p1, 64, 1)
        lhs = jnp.concatenate([
            jnp.where(left8, p1, 0), jnp.where(right8, p2, 0),
            jnp.where(left8, p2, 0), jnp.where(right8, p1, 0)], axis=0)
        ss[pl.ds(SS * (8 * r + k), 64), :] = jnp.dot(
            pltpu.bitcast(lhs, bf16), v_tile(r, k), preferred_element_type=f32)

    def scan(g, r, k, state):
        def s_at(row):
            return ss[pl.ds(SS * 8 * r + row, 8, stride=SS), :]

        seen = []
        if k == 0:
            rows = _span(8 * g, 8, 8)
            seen.append((pr[rows, :], -pi[rows, :]))
            state = (mul[2, rows, :], mul[3, rows, :], s_at(0), -s_at(16))
        cr, ci, xr, xi = state
        for h in range(max(4 * k, 1), 4 * k + 4):
            seen.append((xr, xi))
            base = 32 * (h % 2) + h // 2
            if h < 31:
                xr, xi = ((cr * xr + s_at(base)) + ci * xi,
                          (cr * xi - s_at(base + 16)) - ci * xr)
        for e in range(2):
            for p in range(2):
                zs[r, pl.ds(16 * e + 8 * p + k, 8, stride=ZS), :] = _pack2(
                    seen[e][p], seen[2 + e][p])
        return cr, ci, xr, xi

    def read_out(r, k):
        o = lax.dot_general(pltpu.bitcast(zs[r, pl.ds(ZS * k, 32), :], bf16), v_tile(r, k),
                            NT_DIMS, preferred_element_type=f32)
        ys[r, pl.ds(ZS * k, 16), :] = jnp.where(left16, o[0:16], o[48:64])
        ys[r, pl.ds(ZS * k + 16, 16), :] = jnp.where(left16, o[32:48], o[16:32])

    def taps(g, r):
        ra, rb = pl.ds(0, 8, stride=ZS), pl.ds(16, 8, stride=ZS)
        ya, yb = ys[r, ra, :], ys[r, rb, :]
        ys[r, ra, :], ys[r, rb, :] = jnp.where(left8, 0.0, ya), jnp.where(left8, yb, 0.0)
        kk = jnp.where(left8, ya, yb)
        diag = col[0, _span(8 * g, 8, 8), :]
        ka = pltpu.roll(kk, 1, 1) + pltpu.roll(kk, 65, 1)
        kb = pltpu.roll(kk, 2, 1) + pltpu.roll(kk, 66, 1)
        pos = lane8 & 63
        rs[r] = _pack2(jnp.where(pos == 0, diag, ka),
                       jnp.where(pos == 0, 0.0, jnp.where(pos == 1, diag, kb)))

    def finish(g, r, k, yq, older, acc):
        rb = pltpu.roll(_row(rs, r, k, 32), 0, 1, stride=2, stride_axis=0)
        t = jnp.concatenate([jnp.where(tri0, rb, 0), jnp.where(tri1, rb, 0)], axis=0)
        u = channel(un, g, k, NT // 2)
        for e in range(0 if older is None else 2):
            u = jnp.where(never[e], pltpu.bitcast(older[8 * e:8 * e + 8], i32), u)
        y = jnp.dot(pltpu.bitcast(u, bf16), pltpu.bitcast(t, bf16), preferred_element_type=f32)
        h = y + (channel(xs, g, k, NT) + (yq + ys[r, pl.ds(ZS * k, 16), :]))
        hs[pl.ds(g * 8 + k, NT, stride=HS), :] = h
        if k % 3 == 0:
            fetch(wu_hbm, wu, 7, g, F // 9 * k, F // 3, h[:8])
        return acc[0] + h, acc[1] + h * h, acc[2] + h * _row(col, 1, g * 8 + k, NT)

    def body(g0, q0, steps, carry):
        acc, rolled = carry[0], dict(zip(range(-Q_LAG, 0), carry[1]))
        state = None
        for t in range(steps):
            def at(lag):
                q, k = divmod(t - lag, 8)
                if 0 <= q0 + q < NG:
                    return g0 + q, (q0 + q) % RING, k

            if w := at(LAG_C):
                read_out(*w[1:])
            if w := at(0):
                v = vandermonde(*w)
                if w[2] % 3 == 0 and q0 + t // 8 < 6:
                    fetch(wg_hbm, wg, 6, 8 + w[0], F // 9 * w[2], F // 3, v)
            if w := at(LAG_B):
                state = scan(*w, state)
            if w := at(LAG_A):
                chunk_states(*w)
            if w := at(LAG_D):
                rolled[t] = pltpu.roll(ys[w[1], pl.ds(ZS * w[2] + 16, 16), :], 64, 1)
                acc = finish(*w, rolled[t], rolled.get(t - Q_LAG), acc)
            if (w := at(LAG_K)) and w[2] == 0:
                taps(*w[:2])
        return acc, [rolled[t] for t in range(steps - Q_LAG, steps)]

    zero16 = jnp.zeros((NT, 128), f32)
    fill, n = pl.cdiv(LAG_D + Q_LAG, 8 * RING), NG // RING

    def steady(lo, hi, carry):
        return lax.fori_loop(lo, hi, lambda j, c: body(j * RING, fill * RING, 8 * RING, c),
                             carry, unroll=hi - lo)

    def part(lo, hi, acc):
        carry = (acc, [zero16] * Q_LAG)
        if lo == 0:
            carry, lo = body(0, 0, 8 * RING * fill, (acc, [])), fill
        if min(hi, n) > lo:
            carry = steady(lo, min(hi, n), carry)
        if hi > n:
            carry = body(NG, NG, LAG_D, carry)
        return carry[0]

    acc = (zero16,) * 3
    for lo, hi in zip(CUTS, CUTS[1:]):
        acc = lax.fori_loop(0, 1 + zero, lambda _, c: part(lo, hi, c), acc)

    m2, inv2 = _ln_stats(acc[0], acc[1])
    score = (acc[2] - m2 * jnp.concatenate([vec[2, 0]] * 2)) * inv2
    st2[0], st2[1], st2[2] = m2, inv2, _rnd(score)

    tok = _iota((NT, 128), 0) * 128 + _iota((NT, 128), 1)
    bits = pltpu.bitcast(jnp.where(score == 0.0, 0.0, score), i32) >> 13
    rank = jnp.where(score != score, 0, jnp.where(bits >= 0, bits + (1 << 18), -1 - bits))
    key = pltpu.bitcast((1 << 29) + (rank << 11) + (L - 1 - tok), f32)

    def write_tiles(j, after, WG=3):
        m, s = [[_row(st2, n, 2 * j + e, 8) for e in range(2)] for n in range(2)]
        scale, shift = [v + 1.0 for v in s], [a * b for a, b in zip(m, s)]
        done = [after] * 2
        for q in range(NG):
            if q % WG == 0:
                mult = [jnp.where(never[0], done[-2], v) for v in scale]
            v = [hs[pl.ds((2 * j + e) * HS + 8 * q, 8), :] * mult[e] - shift[e] for e in range(2)]
            ob[pl.ds(8 * q, 8), _lanes(j, 2)] = jnp.concatenate(v, axis=1).astype(bf16)
            if q % 24 == 0 and j < NP:
                fetch(wd_hbm, wd, 9, NG - 1 - j, F // 72 * q, F // 3, v[0])
            if q % WG == WG - 1:
                done.append(v[1])
        return done[-1]

    def send(j):
        for c in (2 * j, 2 * j + 1):
            pl.when(((late >> c) & 1) == 0)(pltpu.make_async_copy(
                ob.at[:, _lanes(c)], o_hbm.at[:, _lanes(c)], sem_o).start)

    def merge(a, b):
        v = a + b[::-1]
        if len(v) > CAP:
            v = [jnp.maximum(p, q) for p, q in zip(v[:CAP], v[CAP:])]
        n = len(v) // 2
        while n:
            v = [jnp.minimum(p, v[i - n]) if i & n else jnp.maximum(p, v[i + n])
                 for i, p in enumerate(v)]
            n //= 2
        return v

    def merge_rows(v):
        for n in (4, 2, 1):
            v = merge(v, [pltpu.roll(p, n, 0) for p in v])
        return v

    def spread(v, shift, stride, after):
        return [jnp.where(never[1], after, pltpu.roll(p, shift, 1, stride=stride, stride_axis=0))
                for p in v]

    tops = merge_rows(merge([key[:8]], [key[8:]]))
    tops = merge_rows(spread(tops, 0, 1, write_tiles(0, tops[0])))
    after = write_tiles(1, tops[0])
    tops = merge_rows(merge(spread(tops, 0, 8, after), spread(tops, 64, 8, after)))
    write_tiles(2, tops[0])
    st2[3] = jnp.where(key >= jnp.concatenate([tops[-1]] * 2), 1.0, 0.0)
    idx = [L - 1 - (pltpu.bitcast(v, i32)[0, 0] & (L - 1)) for v in tops]

    late, fresh = 0, []
    for j in range(CAP):
        fresh.append(((late >> (idx[j] >> 7)) & 1) == 0)
        late = late | (1 << (idx[j] >> 7))

    lane16, row16 = _iota((16, 128), 1), _iota((16, 128), 0)
    tile, lane = [v >> 7 for v in idx], [v & 127 for v in idx]
    stat = [zero16] * 3
    turn, turns = [], 1
    for j in range(CAP):
        pick = ((row16 & 7) == j) & (lane16 == lane[j])
        stat = [jnp.where(pick, _row(st2, n, tile[j], 16), v) for n, v in enumerate(stat)]
        turn.append(sum(jnp.where(lane[i] == lane[j], 1, 0) for i in range(j)))
        turns = jnp.maximum(turns, turn[j] + 1)

    def gather(n, hsel):
        at = [jnp.where(turn[j] == n, lane[j], -1) for j in range(CAP)]
        onehot = zero16
        for j in range(CAP):
            onehot = jnp.where(((row16 & 7) == j) & (lane16 == at[j]), 1.0, onehot)
        merged = []
        for q in range(D // 16):
            v = zero16
            for j in range(CAP):
                v = jnp.where(lane16 == at[j], hs[pl.ds(tile[j] * HS + 16 * q, 16), :], v)
            merged.append(v)
        return hsel + lax.dot_general(
            onehot.astype(bf16), jnp.concatenate(merged, axis=0).astype(bf16),
            NT_DIMS, preferred_element_type=f32)

    hsel = lax.fori_loop(0, turns, gather, jnp.zeros((16, D), f32))
    m_j, s_j, r_j = [jnp.sum(v, axis=1, keepdims=True) for v in stat]
    xsel = _rnd(_rnd(hsel - m_j) * s_j)

    x_main = xsel[:, :512].astype(bf16)
    x_tail = jnp.concatenate([xsel[:, 512:]] * 2, axis=1)
    x_tail = jnp.where((row16 < 8) == (lane16 < 64), x_tail, 0.0).astype(bf16)
    for c in w_cp[:3]:
        c.wait()
    acts, w_t = [], {}

    def transpose_ahead(v):
        n = N_T - 1 - len(w_t)
        if n < 0:
            return v
        w_t[n] = pltpu.bitcast(wd[_lanes(n // (F // 128)), _lanes(n % (F // 128))].T, i32)
        last = pltpu.bitcast(w_t[n][56:], v.dtype)
        return jnp.where(never[n % 2], last + v, v)

    popped = [xsel[:8, :128]] * 2
    for k in range(F // FW):
        f = pl.ds(k * FW, FW)
        x_k = pltpu.bitcast(x_tail, i32)
        for _ in range(TR[k]):
            x_k = transpose_ahead(x_k)
        for j in range(3, NT // 2):
            if WT[j - 3] == k:
                x_k = jnp.where(never[1], pltpu.bitcast(write_tiles(j, popped[-2], WG), i32), x_k)
        for j in range(NT // 2):
            if SD[j] == k:
                send(j)
        tail = jnp.dot(
            pltpu.bitcast(x_k, bf16), jnp.concatenate([wg[pl.ds(512, 64), f], wu[pl.ds(512, 64), f]], axis=0),
            preferred_element_type=f32)
        gate = jnp.dot(x_main, wg[pl.ds(0, 512), f], preferred_element_type=f32)
        up = jnp.dot(x_main, wu[pl.ds(0, 512), f], preferred_element_type=f32)
        popped.append(tail[:8, :128])
        gate, up = _rnd(gate[:8] + tail[:8]), _rnd(up[:8] + tail[8:])
        act = _rnd(gate * jax.nn.sigmoid(gate)) * up
        acts += [act[:, n:n + 128] for n in range(0, FW, 128)]
    weight = _rnd(jax.nn.sigmoid(r_j[:8]))

    routed = [_row(st2, 3, v, 8) > 0 for v in tile]
    w_cp[3].wait()
    clock, ties = 0, []
    for d0 in DO:
        nd = min(128, D - d0)
        rows = pl.ds(d0, nd)
        y = jnp.zeros((8, nd), f32)
        for t in reversed(range(len(acts))):
            n, act = d0 // 128 * len(acts) + t, acts[t]
            clock += 8 if n < N_T or nd < 128 else 16
            while ties and ties[0][0] <= clock:
                act = jnp.where(never[0], ties.pop(0)[1], act)
            if n < N_T:
                y = y + jnp.dot(act.astype(bf16), pltpu.bitcast(w_t[n], bf16),
                                preferred_element_type=f32)
            else:
                y = y + lax.dot_general(act.astype(bf16), wd[rows, _lanes(t)], NT_DIMS,
                                        preferred_element_type=f32)
        new = hsel[:8, d0:d0 + nd] + _rnd(xsel[:8, d0:d0 + nd] + _rnd(_rnd(y) * weight))
        if nd < 128:
            new = jnp.concatenate([new, jnp.zeros((8, 128 - nd), f32)], axis=1)
        for j in range(CAP):
            nb[d0 // 128, pl.ds(idx[j], 1), :] = new[j:j + 1]
        for j in range(CAP):
            cols = _lanes(tile[j])
            one = pltpu.bitcast(nb[d0 // 128, cols, :].astype(bf16).T[:nd], i32)
            for q in range(0, nd, 16):
                lb[j, pl.ds(d0 + q, 16), :] = pltpu.bitcast(jnp.where(
                    routed[j], one[q // 2:q // 2 + 8],
                    pltpu.bitcast(ob[pl.ds(d0 + q, 16), cols], i32)), bf16)
        if TIE[0]:
            ties.append((clock + TIE[0], new))
        ties.append((clock + TIE[1], pltpu.bitcast(one[-8:], f32)))
        ties.sort(key=lambda v: v[0])
        for j in range(CAP):
            pl.when(fresh[j])(pltpu.make_async_copy(
                lb.at[j, rows], o_hbm.at[rows, _lanes(tile[j])], sem_o).start)
    pltpu.make_async_copy(ob, o_hbm, sem_o).wait()


@jax.jit
def pallas_sequential_preLN__ssm_conv_s4__moe_arch_mod__prompt_kernel(
    A_u: jax.Array,
    A_A_re: jax.Array,
    A_A_im: jax.Array,
    A_B_re: jax.Array,
    A_B_im: jax.Array,
    A_C_re: jax.Array,
    A_C_im: jax.Array,
    A_log_dt: jax.Array,
    A_Dskip: jax.Array,
    B_x: jax.Array,
    B_w_r: jax.Array,
    B_w_gate: jax.Array,
    B_w_up: jax.Array,
    B_w_down: jax.Array,
):
    del B_x
    hbm = pl.BlockSpec(memory_space=pltpu.HBM)
    out = pl.pallas_call(
        _kernel,
        out_shape=jax.ShapeDtypeStruct((D, L), bf16),
        in_specs=[hbm] * 13,
        out_specs=hbm,
        scratch_shapes=[
            pltpu.VMEM((D,), bf16),
            pltpu.VMEM((D,), bf16),
            pltpu.VMEM((D,), bf16),
            pltpu.VMEM((6, D, N), bf16),
            pltpu.VMEM((2, D, 128), f32),
            pltpu.VMEM((9 * 584, N), f32),
            pltpu.VMEM((9 * 584, N), f32),
            pltpu.VMEM((6, D, N), f32),
            pltpu.VMEM((3, 5, 8, 128), f32),
            pltpu.VMEM((D, L), bf16),
            pltpu.VMEM((17 * 584, 128), f32),
            pltpu.VMEM((2, NT // 2, 8, 128), f32),
            pltpu.VMEM((9 * 584, 128), i32),
            pltpu.VMEM((9 * 584, 128), i32),
            pltpu.VMEM((RING, 512, N), i32),
            pltpu.VMEM((RING * 8 * SS + 72, N), f32),
            pltpu.VMEM((RING, 8 * ZS + 40, N), i32),
            pltpu.VMEM((RING, 8 * ZS + 40, 128), f32),
            pltpu.VMEM((RING, 8, 128), i32),
            pltpu.VMEM((17 * 584, 128), f32),
            pltpu.VMEM((4, NT, 128), f32),
            pltpu.VMEM((D, L), bf16),
            pltpu.VMEM((CAP, D, 128), bf16),
            pltpu.VMEM((5, L, 128), f32),
            pltpu.VMEM((D, F), bf16),
            pltpu.VMEM((D, F), bf16),
            pltpu.VMEM((D, F), bf16),
            pltpu.SemaphoreType.DMA((10,)),
            pltpu.SemaphoreType.DMA(()),
        ],
        compiler_params=pltpu.CompilerParams(
            vmem_limit_bytes=100 * 1024 * 1024,
            flags={"XLA_TPU_FORCE_LP_LLO_SCHEDULER": True},
        ),
    )(
        A_u.reshape(L, D).T, A_A_re, A_A_im, A_B_re, A_B_im, A_C_re, A_C_im,
        A_log_dt, A_Dskip, B_w_r, B_w_gate, B_w_up, B_w_down.T,
    )
    return out.T.reshape(1, L, D)
```

```python
import jax
import jax.numpy as jnp
from jax import lax
import jax.experimental.pallas as pl
import jax.experimental.pallas.tpu as pltpu

D = 576
L = 2048
N = 128
F = 4608
CAP = 8
EPS = 1e-5

NT = L // 128
NG = D // 8

HS = 580
PS = 577
SS = 65
ZS = 36

RING = 4
LAG_A, LAG_B, LAG_C, LAG_K, LAG_D = 0, 16, 24, 42, 48
Q_LAG = 4
N_T = 88
PARTS = (0, 6, 16, 36)
SU = 3
PB = 16
PU = 4
XW = 256
XQ = 33
ALT = 8
MU = 8
XP = 896
NP = 3
XG = 0
FG = ()
NQ = 3
ALLW = 0
WP = 16
DW = 1
DA = 384
FK3 = (0, 3, 6)
DQ = 48
FK = 1.0
ORDER = 'CVBAKD'
TIE = (150, 550)
DO = (0, 128, 256, 384, 512)
TR = (0, 4, 12, 12, 12, 12, 12, 12, 12)
WT = (-1, -1, 4, 6, 8)
WG = 1
SD = (4,) * 6 + (6, 8)
CUTS = (0, 9, 18, 19)
FW = 512

f32 = jnp.float32
bf16 = jnp.bfloat16
i32 = jnp.int32
NT_DIMS = (((1,), (1,)), ((), ()))


def _rnd(x):
    return x.astype(bf16).astype(f32)


def _cmul(ar, ai, br, bi):
    return ar * br - ai * bi, ar * bi + ai * br


def _csq(ar, ai):
    t = ar * ai
    return ar * ar - ai * ai, t + t


def _csqrt(wr, wi):
    big = jnp.clip(jnp.maximum(jnp.abs(wr), jnp.abs(wi)), 2.0 ** -125, 2.0 ** 125)
    e = jnp.log2(big)
    down = jnp.exp2(-e)
    xr, xi = wr * down, wi * down
    p = jnp.exp2(0.5 * jnp.log2(xr * xr + xi * xi)) + jnp.abs(xr)
    q = jnp.exp2(0.5 * ((e - 1.0) - jnp.log2(jnp.maximum(p, 2.0 ** -60))))
    t, o = p * q, xi * q
    pos = xr >= 0
    return jnp.where(pos, t, o), jnp.where(pos, o, t)


def _unpack2(w):
    return pltpu.bitcast(w << 16, f32), pltpu.bitcast(w & (-65536), f32)


def _interleave(a, b):
    return jnp.concatenate([a, b], axis=1).astype(bf16).reshape(2 * a.shape[0], 128)


def _pack2(a, b):
    return pltpu.bitcast(_interleave(a, b), i32)


def _ln_stats(s1, s2):
    m = s1 * (1.0 / D)
    v = _rnd(jnp.maximum(s2 * (1.0 / D) - m * m, 0.0))
    return _rnd(m), 1.0 / _rnd(jnp.sqrt(_rnd(v + _rnd(jnp.full_like(v, EPS)))))


def _span(start, size, align):
    return pl.ds(start if isinstance(start, int) else pl.multiple_of(start, align), size)


def _lanes(c, n=1):
    return _span(128 * n * c, 128 * n, 128 * n)


def _row(ref, k, r, rows):
    return jnp.broadcast_to(ref[k, pl.ds(r, 1), :], (rows, 128))


def _iota(shape, axis):
    return lax.broadcasted_iota(i32, shape, axis)


def _main(
    x_hbm, are_hbm, aim_hbm, bre_hbm, bim_hbm, cre_hbm, cim_hbm,
    ldt_hbm, dsk_hbm, wr_hbm, wg_hbm, wu_hbm, wd_hbm,
    o_hbm,
    ldt, dsk, wrt, prm, col, pr, pi, mul, vec, xb, xs, st1, un, ur,
    vs, ss, zs, ys, rs, hs, st2, ob, nb, wg, wu, wd, we, lb,
    sem_o, sem_p,
):
    we_hbm = wd_hbm.at[pl.ds(DA, D - DA)]

    def p_cp(j):
        rows = pl.ds(16 * PARTS[j], 16 * (PARTS[j + 1] - PARTS[j]))
        return [pltpu.make_async_copy(src.at[rows], prm.at[k, rows], sem_p.at[1 + j])
                for k, src in enumerate((are_hbm, aim_hbm, bre_hbm, bim_hbm, cre_hbm, cim_hbm))]

    def copy(src, dst, sem, rows=slice(None), cols=slice(None)):
        return pltpu.make_async_copy(src.at[rows, cols], dst.at[rows, cols], sem_p.at[sem])

    def fetch(src, dst, sem, i, c0, width, after, n=8):
        rows = _span(8 * i, 8, 8)
        dst[rows, pl.ds(c0, 128)] = after.astype(bf16)
        copy(src, dst, sem, _span(8 * i, n, 8), pl.ds(c0, width)).start()

    v_cp = [pltpu.make_async_copy(a, b, sem_p.at[0])
            for a, b in ((ldt_hbm, ldt), (dsk_hbm, dsk), (wr_hbm, wrt))]
    x_cp = [copy(x_hbm, xb, 4, pl.ds(0, XW)), copy(x_hbm, xb, 5, pl.ds(XW, D - XW))]
    w_cp = [copy(wg_hbm, wg, 6), copy(wu_hbm, wu, 7),
            copy(wd_hbm, wd, 8, pl.ds(0, DA)), copy(we_hbm, we, 9)]
    for k, c in enumerate(v_cp + sum([p_cp(j) for j in range(len(PARTS) - 1)], []) + [
            x_cp[0], copy(x_hbm, xb, 5, pl.ds(XW, D - 8 * XQ - XW)),
            copy(wg_hbm, wg, 6, cols=pl.ds(XG, F - XG)), copy(wd_hbm, wd, 8, pl.ds(64, DA - 64)),
            copy(we_hbm, we, 9, pl.ds(0, D - DA - 8 * (NP + NQ) - 48))]):
        c.start(priority=int(k > ALT or k % 2))

    lane8, sub8 = _iota((8, 128), 1), _iota((8, 128), 0)

    def lane_sum(v):
        return jnp.broadcast_to(jnp.sum(v, axis=1, keepdims=True), (8, 128))

    for c in v_cp:
        c.wait()
    for k, ref in enumerate((ldt, dsk, wrt)):
        row = ref[...].astype(f32).reshape(1, D)
        row = jnp.concatenate([row, jnp.zeros((1, 640 - D), f32)], axis=1)
        for t in range(5):
            v = jnp.broadcast_to(row[:, 128 * t:128 * t + 128], (8, 128))
            vec[k, t] = v if k else _rnd(jnp.exp(v))

    def own(k, g):
        return jnp.where(lane8 - sub8 == 8 * (g & 15), vec[k, g >> 4], 0.0)

    @pl.loop(0, NG, unroll=NG)
    def _(g):
        col[2, _span(8 * g, 8, 8), :] = lane_sum(own(0, g))

    vec[0, 0] = lane_sum(sum(vec[2, t] for t in range(5)))

    def opaque_zero(v):
        return jnp.minimum(pltpu.bitcast(v, i32)[0, 0] & 1, 0)

    zero = opaque_zero(vec[1, 0])
    never = (lane8 < zero, sub8 < zero)

    def step(g, *after):
        rows = _span(8 * g, 8, 8)
        dt = col[2, rows, :]
        for mask, v in zip(never, after):
            dt = jnp.where(mask, v, dt)
        mag, ph = jnp.exp(dt * prm[0, rows, :].astype(f32)), dt * prm[1, rows, :].astype(f32)
        cos = jnp.cos(ph)
        mul[4, rows, :], mul[5, rows, :] = mag * cos, mag * jnp.sin(ph)
        return mag, cos

    def powers(g, after):
        rows = _span(8 * g, 8, 8)
        dt = jnp.where(never[0], after, col[2, rows, :])
        br, bi, cr, ci = [prm[k, rows, :].astype(f32) for k in range(2, 6)]
        w = _cmul(cr, ci, dt * br, dt * bi)
        col[0, rows, :] = lane_sum(w[0] + own(1, g))
        col[1, rows, :] = lane_sum(own(2, g))
        a = mul[4, rows, :], mul[5, rows, :]
        v = _csqrt(*_cmul(*w, *a))
        a = _csq(*a)
        for j in range(8):
            pr[pl.ds(j * PS + rows.start, 8), :], pi[pl.ds(j * PS + rows.start, 8), :] = v
            last, v = v[0], _cmul(*v, *a)
        for _ in range(3):
            a = _csq(*a)
        mul[0, rows, :], mul[1, rows, :] = a
        mul[2, rows, :], mul[3, rows, :] = _csq(*_csq(*a))
        return last

    def set_up(lo, hi, carry):
        def one(g, carry):
            trig, done = carry
            mag = cos = last = trig[0]
            if lo < NG:
                mag, cos = step(g, trig[0], done[0])
            if lo < 2 * XQ:
                fetch(x_hbm, xb, 5, NG - XQ + (g >> 1), pl.multiple_of(L // 2 * (g & 1), L // 2),
                      L // 2, mag)
            if lo >= SU:
                last = powers(g - SU, trig[0])
            return trig[1:] + [cos], done[1:] + [last]

        return lax.fori_loop(lo, hi, one, carry, unroll=hi - lo)

    carry = tuple([jnp.zeros((8, 128), f32)] * k for k in (SU, PU))
    cuts = sorted([2 * v for v in PARTS] + [SU, 2 * XQ, NG + SU])
    for lo, hi in zip(cuts, cuts[1:]):
        for j, v in enumerate(PARTS[:-1]):
            for c in p_cp(j) if lo == 2 * v else []:
                c.wait()
        carry = set_up(lo, hi, carry)

    def moments(i, lo, hi, after):
        s1 = s2 = jnp.concatenate([jnp.where(never[0], after, 0.0)] * 2, axis=1)
        if lo:
            s1, s2 = st1[i, 0], st1[i, 1]
        for q in range(lo, hi, 8):
            v = xb[pl.ds(q, 8), _lanes(i, 2)].astype(f32)
            for e in range(2):
                xs[pl.ds((2 * i + e) * HS + q, 8), :] = v[:, 128 * e:128 * e + 128]
            s1, s2 = s1 + v, s2 + v * v
        fetch(wd_hbm, wd, 8, i, F // 3 * (lo > 0), F // 3, v[:, :128])
        if lo:
            s1, s2 = [jnp.broadcast_to(jnp.sum(v, axis=0, keepdims=True), v.shape) for v in (s1, s2)]
            s1, s2 = _ln_stats(s1, s2)
        st1[i, 0], st1[i, 1] = s1, s2
        return s2[:, :128]

    flip = jnp.where(_iota((128, 128), 0) == _iota((128, 128), 1) ^ 63, 1.0, 0.0).astype(bf16)

    def normalise(i):
        m, s = [[st1[i, n, :, _lanes(e)] for e in range(2)] for n in range(2)]
        for q in range(D // 16):
            xa, xc = [[xs[pl.ds(c * HS + 16 * q + 8 * e, 8), :] for e in range(2)]
                      for c in (2 * i, 2 * i + 1)]
            u = [((xa[e] - m[0]) * s[0], (xc[e] - m[1]) * s[1]) for e in range(2)]
            w = [_pack2(*v) for v in u]
            if q % 3 == 0:
                r = jnp.dot(jnp.concatenate(u[0] + u[1], axis=0).astype(bf16), flip,
                            preferred_element_type=f32)
                r = [_pack2(r[n:n + 8], r[n + 8:n + 16]) for n in (0, 16)]
            else:
                r = [jnp.take_along_axis(v, lane8 ^ 63, axis=1, mode="promise_in_bounds")
                     for v in w]
            for e in range(2):
                rows = pl.ds(i * HS + 16 * q + 8 * e, 8)
                un[rows, :], ur[rows, :] = w[e], r[e]
        fetch(wd_hbm, wd, 8, i, F // 3 * 2, F // 3, u[0][0])

    left8, right8 = lane8 < 64, lane8 >= 64
    left16 = _iota((16, 128), 1) < 64
    lane32, row32 = _iota((32, 128), 1), 2 * _iota((32, 128), 0)
    tri0, tri1 = (lane32 >= row32) & (lane32 < 64), lane32 >= row32 + 64

    def v_tile(r, k):
        return pltpu.bitcast(vs[r, pl.ds(64 * k, 64), :], bf16)

    def channel(ref, g, k, n):
        return ref[pl.ds(g * 8 + k, n, stride=HS), :]

    def vandermonde(g, r, k):
        ch = g * 8 + k
        vr, vi = pr[pl.ds(ch, 8, stride=PS), :], pi[pl.ds(ch, 8, stride=PS), :]
        odd = _cmul(vr, vi, _row(mul, 4, ch, 8), _row(mul, 5, ch, 8))
        vr, vi = jnp.concatenate([vr, odd[0]], axis=0), jnp.concatenate([vi, odd[1]], axis=0)
        mr, mi = _row(mul, 0, ch, 16), _row(mul, 1, ch, 16)
        re, im = [], []
        for q in range(4):
            re.append(_pack2(vr[:8], vr[8:]))
            im.append(_pack2(vi[:8], vi[8:]))
            vr, vi = _cmul(vr, vi, mr, mi)
        for q, v in enumerate(re + im):
            vs[r, pl.ds(64 * k + 8 * q, 8), :] = v
        return odd[0]


    @pl.loop(0, 1 + zero)
    def _(_):
        for c, lo, hi in zip(x_cp, (0, XW), (XW, D)):
            c.wait()
            lax.fori_loop(0, NT // 2, lambda i, v: moments(i, lo, hi, v), jnp.zeros((8, 128), f32),
                          unroll=NT // 2)
        pl.loop(0, NT // 2, unroll=NT // 2)(normalise)

    def chunk_states(g, r, k):
        p1 = channel(ur, g, k, NT // 2)
        p2 = pltpu.roll(p1, 64, 1)
        lhs = jnp.concatenate([
            jnp.where(left8, p1, 0), jnp.where(right8, p2, 0),
            jnp.where(left8, p2, 0), jnp.where(right8, p1, 0)], axis=0)
        ss[pl.ds(SS * (8 * r + k), 64), :] = jnp.dot(
            pltpu.bitcast(lhs, bf16), v_tile(r, k), preferred_element_type=f32)

    def scan(g, r, k, state):
        def s_at(row):
            return ss[pl.ds(SS * 8 * r + row, 8, stride=SS), :]

        seen = []
        if k == 0:
            rows = _span(8 * g, 8, 8)
            seen.append((pr[rows, :], -pi[rows, :]))
            state = (mul[2, rows, :], mul[3, rows, :], s_at(0), -s_at(16))
        cr, ci, xr, xi = state
        for h in range(max(4 * k, 1), 4 * k + 4):
            seen.append((xr, xi))
            base = 32 * (h % 2) + h // 2
            if h < 31:
                xr, xi = ((cr * xr + s_at(base)) + ci * xi,
                          (cr * xi - s_at(base + 16)) - ci * xr)
        for e in range(2):
            for p in range(2):
                zs[r, pl.ds(16 * e + 8 * p + k, 8, stride=ZS), :] = _pack2(
                    seen[e][p], seen[2 + e][p])
        return cr, ci, xr, xi

    def read_out(r, k, y):
        o = lax.dot_general(pltpu.bitcast(zs[r, pl.ds(ZS * k, 32), :], bf16), v_tile(r, k),
                            NT_DIMS, preferred_element_type=f32)
        ys[y, pl.ds(ZS * k, 16), :] = jnp.where(left16, o[0:16], o[48:64])
        ys[y, pl.ds(ZS * k + 16, 16), :] = jnp.where(left16, o[32:48], o[16:32])

    def taps(g, r):
        ra, rb = pl.ds(0, 8, stride=ZS), pl.ds(16, 8, stride=ZS)
        ya, yb = ys[r, ra, :], ys[r, rb, :]
        ys[r, ra, :], ys[r, rb, :] = jnp.where(left8, 0.0, ya), jnp.where(left8, yb, 0.0)
        kk = jnp.where(left8, ya, yb)
        diag = col[0, _span(8 * g, 8, 8), :]
        ka = pltpu.roll(kk, 1, 1) + pltpu.roll(kk, 65, 1)
        kb = pltpu.roll(kk, 2, 1) + pltpu.roll(kk, 66, 1)
        pos = lane8 & 63
        rs[r] = _pack2(jnp.where(pos == 0, diag, ka),
                       jnp.where(pos == 0, 0.0, jnp.where(pos == 1, diag, kb)))

    def pace(g, k, after):
        if k in FK3:
            fetch(wu_hbm, wu, 7, g, F // len(FK3) * FK3.index(k), F // len(FK3), after)
        if XG and k in FG:
            fetch(wg_hbm, wg, 6, g, XG // len(FG) * FG.index(k), XG // len(FG), after)

    def finish(g, r, k, yq, older, acc):
        rb = pltpu.roll(_row(rs, r, k, 32), 0, 1, stride=2, stride_axis=0)
        t = jnp.concatenate([jnp.where(tri0, rb, 0), jnp.where(tri1, rb, 0)], axis=0)
        u = channel(un, g, k, NT // 2)
        for e in range(0 if older is None else 2):
            u = jnp.where(never[e], pltpu.bitcast(older[8 * e:8 * e + 8], i32), u)
        y = jnp.dot(pltpu.bitcast(u, bf16), pltpu.bitcast(t, bf16), preferred_element_type=f32)
        h = y + (channel(xs, g, k, NT) + (yq + ys[r, pl.ds(ZS * k, 16), :]))
        hs[pl.ds(g * 8 + k, NT, stride=HS), :] = h
        if isinstance(g, int) and g >= NG - 6:
            if k % 3 == 0:
                fetch(we_hbm, we, 9, g - DA // 8, F // 9 * k, F // 3, h[:8])
        else:
            pace(g, k, h[:8])
        return acc[0] + h, acc[1] + h * h, acc[2] + h * _row(col, 1, g * 8 + k, NT)

    def body(g0, q0, steps, carry):
        acc, rolled = carry[0], dict(zip(range(-Q_LAG, 0), carry[1]))
        state = None
        for t in range(steps):
            def at(lag):
                q, k = divmod(t - lag, 8)
                if 0 <= q0 + q < NG:
                    return g0 + q, (q0 + q) % RING, k

            for stage in ORDER:
                if stage == "C" and (w := at(LAG_C)):
                    read_out(*w[1:], w[1])
                if stage == "V" and (w := at(0)):
                    v = vandermonde(*w)
                    if q0 + t // 8 < 6:
                        pace(NG - 6 + w[0], w[2], v)
                if stage == "B" and (w := at(LAG_B)):
                    state = scan(*w, state)
                if stage == "A" and (w := at(LAG_A)):
                    chunk_states(*w)
                if stage == "D" and (w := at(LAG_D)):
                    rolled[t] = pltpu.roll(ys[w[1], pl.ds(ZS * w[2] + 16, 16), :], 64, 1)
                    acc = finish(*w, rolled[t], rolled.get(t - Q_LAG), acc)
                if stage == "K" and (w := at(LAG_K)) and w[2] == 0:
                    taps(*w[:2])
        return acc, [rolled[t] for t in range(steps - Q_LAG, steps)]

    zero16 = jnp.zeros((NT, 128), f32)
    fill, n = pl.cdiv(LAG_D + Q_LAG, 8 * RING), NG // RING

    def steady(lo, hi, carry):
        return lax.fori_loop(lo, hi, lambda j, c: body(j * RING, fill * RING, 8 * RING, c),
                             carry, unroll=hi - lo)

    def drain(acc):
        def left(lag):
            return [(ch // 8, ch // 8 % RING, ch % 8) for ch in range(D - lag, D)]

        for w in left(LAG_A):
            chunk_states(*w)
        state = None
        for w in left(LAG_B):
            state = scan(*w, state)
        todo = {"C": left(LAG_C), "D": left(LAG_D), "K": [w for w in left(LAG_K) if w[2] == 0]}
        rolled = [None] * DQ
        for stage in ("C" * (LAG_C - 24) + "K" * (len(todo["K"]) - 3) + "C" * 24
                      + "D" * (LAG_D - 32) + "KKK" + "D" * 32):
            g, r, k = todo[stage].pop(0)
            w = g, r if g < NG - 2 else r + 2, k
            if stage == "C":
                read_out(r, k, w[1])
            elif stage == "K":
                taps(*w[:2])
            else:
                rolled.append(pltpu.roll(ys[w[1], pl.ds(ZS * w[2] + 16, 16), :], 64, 1))
                acc = finish(*w, rolled[-1], rolled[-1 - DQ], acc)
        assert not any(todo.values())
        return acc

    def part(lo, hi, acc):
        carry = (acc, [zero16] * Q_LAG)
        if lo == 0:
            carry, lo = body(0, 0, 8 * RING * fill, (acc, [])), fill
        if min(hi, n) > lo:
            carry = steady(lo, min(hi, n), carry)
        if hi > n:
            return drain(carry[0])
        return carry[0]

    acc = (zero16,) * 3
    for lo, hi in zip(CUTS, CUTS[1:]):
        acc = lax.fori_loop(0, 1 + zero, lambda _, c: part(lo, hi, c), acc)
    m2, inv2 = _ln_stats(acc[0], acc[1])
    score = (acc[2] - m2 * jnp.concatenate([vec[0, 0]] * 2)) * inv2
    st2[0], st2[1], st2[2] = m2, inv2, _rnd(score)

    tok = _iota((NT, 128), 0) * 128 + _iota((NT, 128), 1)
    bits = pltpu.bitcast(jnp.where(score == 0.0, 0.0, score), i32) >> 13
    rank = jnp.where(score != score, 0, jnp.where(bits >= 0, bits + (1 << 18), -1 - bits))
    key = pltpu.bitcast((1 << 29) + (rank << 11) + (L - 1 - tok), f32)

    def write_tiles(j, after, WG=3):
        m, s = [[_row(st2, n, 2 * j + e, 8) for e in range(2)] for n in range(2)]
        scale, shift = [v + 1.0 for v in s], [a * b for a, b in zip(m, s)]
        done = [after] * 2
        for q in range(NG):
            if q % WG == 0:
                mult = [jnp.where(never[0], done[-2], v) for v in scale]
            v = [hs[pl.ds((2 * j + e) * HS + 8 * q, 8), :] * mult[e] - shift[e] for e in range(2)]
            ob[pl.ds(8 * q, 8), _lanes(j, 2)] = jnp.concatenate(v, axis=1).astype(bf16)
            if q % 24 == 0 and j < NP:
                fetch(we_hbm, we, 9, NG - DA // 8 - 7 - j, F // 72 * q, F // 3, v[0])
            if q % WG == WG - 1:
                done.append(v[1])
        return done[-1]

    def send(j, after=None):
        none = 0 if after is None else opaque_zero(after)
        for c in (2 * j, 2 * j + 1):
            pl.when(((late >> c) & 1) == none)(lambda: pltpu.make_async_copy(
                ob.at[:, _lanes(c)], o_hbm.at[:, _lanes(c)], sem_o).start(priority=c % 2))

    def merge(a, b):
        v = a + b[::-1]
        if len(v) > CAP:
            v = [jnp.maximum(p, q) for p, q in zip(v[:CAP], v[CAP:])]
        n = len(v) // 2
        while n:
            v = [jnp.minimum(p, v[i - n]) if i & n else jnp.maximum(p, v[i + n])
                 for i, p in enumerate(v)]
            n //= 2
        return v

    def merge_rows(v):
        for n in (4, 2, 1):
            v = merge(v, [pltpu.roll(p, n, 0) for p in v])
        return v

    def spread(v, shift, stride, after):
        return [jnp.where(never[1], after, pltpu.roll(p, shift, 1, stride=stride, stride_axis=0))
                for p in v]

    tops = merge_rows(merge([key[:8]], [key[8:]]))
    tops = merge_rows(spread(tops, 0, 1, write_tiles(0, tops[0])))
    after = write_tiles(1, tops[0])
    tops = merge_rows(merge(spread(tops, 0, 8, after), spread(tops, 64, 8, after)))
    write_tiles(2, tops[0])
    st2[3] = jnp.where(key >= jnp.concatenate([tops[-1]] * 2), 1.0, 0.0)
    idx = [L - 1 - (pltpu.bitcast(v, i32)[0, 0] & (L - 1)) for v in tops]


    lane16, row16 = _iota((16, 128), 1), _iota((16, 128), 0)
    tile, lane = [v >> 7 for v in idx], [v & 127 for v in idx]
    turn, turns = [], 1
    for j in range(CAP):
        turn.append(sum(jnp.where(lane[i] == lane[j], 1, 0) for i in range(j)))
        turns = jnp.maximum(turns, turn[j] + 1)

    def gather(n, carry):
        at = [jnp.where(turn[j] == n, lane[j], -1) for j in range(CAP)]
        onehot = zero16[:8]
        for j in range(CAP):
            onehot = jnp.where((sub8 == j) & (lane8 == at[j]), 1.0, onehot)
        merged = []
        for q in range(D // 16):
            v = zero16
            for j in range(CAP):
                v = jnp.where(lane16 == at[j], hs[pl.ds(tile[j] * HS + 16 * q, 16), :], v)
            merged.append(v)
        after = v[:8]
        for j in range(3, NT // 2):
            if WT[j - 3] < 0:
                after = write_tiles(j, after)
        merged = jnp.concatenate(merged + merged[-4:], axis=0).astype(bf16)
        stat = [zero16[:8]] * 3
        for j in range(CAP):
            pick = (sub8 == j) & (lane8 == at[j])
            stat = [jnp.where(pick, _row(st2, k, tile[j], 8), v) for k, v in enumerate(stat)]
        rows = lax.dot_general(onehot.astype(bf16), merged, NT_DIMS, preferred_element_type=f32)
        return [a + b for a, b in zip(carry, [rows] + [lane_sum(v) for v in stat])]

    hsel, m_j, s_j, r_j = lax.fori_loop(0, turns, gather,
                                        [jnp.zeros((8, 640), f32)] + [zero16[:8]] * 3)
    xsel = _rnd(_rnd(hsel - jnp.tile(m_j, (1, 5))) * jnp.tile(s_j, (1, 5)))

    x_main = xsel[:, :512].astype(bf16)
    x_tail = jnp.concatenate([xsel[:, 512:]] * 2, axis=0)
    x_tail = jnp.where((row16 < 8) == (lane16 < 64), x_tail, 0.0).astype(bf16)
    for c in w_cp[:3]:
        c.wait()
    late, fresh = 0, []
    for j in range(CAP):
        fresh.append(((late >> (idx[j] >> 7)) & 1) == 0)
        late = late | (1 << (idx[j] >> 7))
    acts, w_t = [], {}

    def transpose_ahead(v):
        n = N_T - 1 - len(w_t)
        if n < 0:
            return v
        w_t[n] = pltpu.bitcast(wd[_lanes(n // (F // 128)), _lanes(n % (F // 128))].T, i32)
        last = pltpu.bitcast(w_t[n][56:], v.dtype)
        return jnp.where(never[n % 2], last + v, v)

    popped = [xsel[:8, :128]] * 2
    for k in range(F // FW):
        f = pl.ds(k * FW, FW)
        x_k = pltpu.bitcast(x_tail, i32)
        for _ in range(TR[k]):
            x_k = transpose_ahead(x_k)
        for j in range(3, NT // 2):
            if WT[j - 3] == k:
                x_k = jnp.where(never[1], pltpu.bitcast(write_tiles(j, popped[-2], WG), i32), x_k)
        for j in range(NT // 2):
            if SD[j] == k:
                send(j)
        tail = jnp.dot(
            pltpu.bitcast(x_k, bf16), jnp.concatenate([wg[pl.ds(512, 64), f], wu[pl.ds(512, 64), f]], axis=0),
            preferred_element_type=f32)
        gate = jnp.dot(x_main, wg[pl.ds(0, 512), f], preferred_element_type=f32)
        up = jnp.dot(x_main, wu[pl.ds(0, 512), f], preferred_element_type=f32)
        popped.append(tail[:8, :128])
        for j in range(NT // 2):
            if SD[j] - k in (0.25, 0.5, 0.75):
                send(j, (tail, gate, up)[int(4 * (SD[j] - k)) - 1][:8, :128])
        for e, v in enumerate((tail, gate, up) if k < NQ else ()):
            fetch(we_hbm, we, 9, NG - DA // 8 - 7 - NP - k, F // 3 * e, F // 3, v[:8, :128])
        gate, up = _rnd(gate[:8] + tail[:8]), _rnd(up[:8] + tail[8:])
        act = _rnd(gate * jax.nn.sigmoid(gate)) * up
        acts += [act[:, n:n + 128] for n in range(0, FW, 128)]
    weight = _rnd(jax.nn.sigmoid(r_j[:8]))

    routed = [_row(st2, 3, v, 8) > 0 for v in tile]
    clock, ties, after = 0, [], weight
    for j in range(NT // 2):
        if j >= 3 and WT[j - 3] > 8:
            after = write_tiles(j, after, 2)
            ties.append((WT[j - 3], after))
        if SD[j] >= 9:
            send(j)
    def patch(d0, y):
        nd = y.shape[1]
        rows = pl.ds(d0, nd)
        new = hsel[:8, d0:d0 + nd] + _rnd(xsel[:8, d0:d0 + nd] + _rnd(_rnd(y) * weight[:, :nd]))
        if nd < 128:
            new = jnp.concatenate([new, jnp.zeros((8, 128 - nd), f32)], axis=1)
        for j in range(CAP):
            nb[d0 // 64, pl.ds(idx[j], 1), :] = new[j:j + 1]
        for j in range(CAP):
            cols = _lanes(tile[j])
            one = pltpu.bitcast(nb[d0 // 64, cols, :].astype(bf16).T[:nd], i32)
            for q in range(0, nd, 16):
                lb[j][pl.ds(d0 + q, 16), :] = pltpu.bitcast(jnp.where(
                    routed[j], one[q // 2:q // 2 + 8],
                    pltpu.bitcast(ob[pl.ds(d0 + q, 16), cols], i32)), bf16)
        if TIE[0]:
            ties.append((clock + TIE[0], new))
        ties.append((clock + TIE[1], pltpu.bitcast(one[-8:], f32)))
        ties.sort(key=lambda v: v[0])
        for j in range(CAP):
            pl.when(fresh[j])(lambda: pltpu.make_async_copy(
                lb[j].at[rows], o_hbm.at[rows, _lanes(tile[j])], sem_o).start(priority=j % 2))

    held = []
    for d0 in DO:
        nd = min(v - d0 for v in DO + (D,) if v > d0)
        rows = pl.ds(d0, nd)
        y = jnp.zeros((8, nd), f32)
        for t in reversed(range(len(acts))):
            n, act = d0 // 128 * len(acts) + t, acts[t]
            clock += 8 if n < N_T else nd // 8
            while ties and ties[0][0] <= clock:
                act = jnp.where(never[0], ties.pop(0)[1], act)
            if n < N_T:
                y = y + jnp.dot(act.astype(bf16), pltpu.bitcast(w_t[n], bf16),
                                preferred_element_type=f32)
            else:
                y = y + lax.dot_general(act.astype(bf16), wd[rows, _lanes(t)] if d0 < DA else we[pl.ds(d0 - DA, nd), _lanes(t)], NT_DIMS,
                                        preferred_element_type=f32)
        held.append((d0, y))
        if d0 == DO[2]:
            w_cp[3].wait()
            ties.clear()
            clock -= 200
        while held and (d0 != DO[1] or DW):
            patch(*held.pop(0))


def _kernel(*refs):
    pl.run_scoped(lambda sem: _main(*refs, sem), pltpu.SemaphoreType.DMA((10,)))
    pltpu.make_async_copy(refs[13], refs[13], refs[-1]).wait()


@jax.jit
def pallas_sequential_preLN__ssm_conv_s4__moe_arch_mod__prompt_kernel(
    A_u: jax.Array,
    A_A_re: jax.Array,
    A_A_im: jax.Array,
    A_B_re: jax.Array,
    A_B_im: jax.Array,
    A_C_re: jax.Array,
    A_C_im: jax.Array,
    A_log_dt: jax.Array,
    A_Dskip: jax.Array,
    B_x: jax.Array,
    B_w_r: jax.Array,
    B_w_gate: jax.Array,
    B_w_up: jax.Array,
    B_w_down: jax.Array,
):
    del B_x
    hbm = pl.BlockSpec(memory_space=pltpu.HBM)
    out = pl.pallas_call(
        _kernel,
        out_shape=jax.ShapeDtypeStruct((D, L), bf16),
        in_specs=[hbm] * 13,
        out_specs=hbm,
        scratch_shapes=[
            pltpu.VMEM((D,), bf16),
            pltpu.VMEM((D,), bf16),
            pltpu.VMEM((D,), bf16),
            pltpu.VMEM((6, D, N), bf16),
            pltpu.VMEM((3, D, 128), f32),
            pltpu.VMEM((9 * 584, N), f32),
            pltpu.VMEM((9 * 584, N), f32),
            pltpu.VMEM((6, D, N), f32),
            pltpu.VMEM((3, 5, 8, 128), f32),
            pltpu.VMEM((D, L), bf16),
            pltpu.VMEM((17 * 584, 128), f32),
            pltpu.VMEM((NT // 2, 2, 8, 256), f32),
            pltpu.VMEM((9 * 584, 128), i32),
            pltpu.VMEM((9 * 584, 128), i32),
            pltpu.VMEM((RING, 512, N), i32),
            pltpu.VMEM((RING * 8 * SS + 72, N), f32),
            pltpu.VMEM((RING, 8 * ZS + 40, N), i32),
            pltpu.VMEM((RING + 2, 8 * ZS + 40, 128), f32),
            pltpu.VMEM((RING + 2, 8, 128), i32),
            pltpu.VMEM((17 * 584, 128), f32),
            pltpu.VMEM((4, NT, 128), f32),
            pltpu.VMEM((D, L), bf16),
            pltpu.VMEM((9, L, 128), f32),
            pltpu.VMEM((D, F), bf16),
            pltpu.VMEM((D, F), bf16),
            pltpu.VMEM((DA, F), bf16),
            pltpu.VMEM((D - DA, F), bf16),
            [pltpu.VMEM((D, 128), bf16)] * CAP,
            pltpu.SemaphoreType.DMA(()),
        ],
        compiler_params=pltpu.CompilerParams(
            vmem_limit_bytes=100 * 1024 * 1024,
            flags={"XLA_TPU_FORCE_LP_LLO_SCHEDULER": True},
        ),
    )(
        A_u.reshape(L, D).T, A_A_re, A_A_im, A_B_re, A_B_im, A_C_re, A_C_im,
        A_log_dt, A_Dskip, B_w_r, B_w_gate, B_w_up, B_w_down.T,
    )
    return out.T.reshape(1, L, D)
```

```python
import jax
import jax.numpy as jnp
from jax import lax
import jax.experimental.pallas as pl
import jax.experimental.pallas.tpu as pltpu

D = 576
L = 2048
N = 128
F = 4608
CAP = 8
EPS = 1e-5

NT = L // 128
NG = D // 8
DB = D // 3

HS = 580
PS = 577
SS = 65
ZS = 36

PARTS = (0, 12, 32, NG)
X_ROWS = (112, 312, 488)
RING = 4
LAG_B, LAG_C, LAG_K, LAG_D = 16, 24, 42, 48
Q_LAG = 4
FW = 512
GW = 1024
TR = (0, 4, 12, 12, 12, 12, 12, 12, 12)
WT = {3: 5, 5: 6, 7: 7}
NQ = 2
RU = 6
TIE = (24, 34)
TN = 12

f32 = jnp.float32
bf16 = jnp.bfloat16
i32 = jnp.int32
NT_DIMS = (((1,), (1,)), ((), ()))


def _rnd(x):
    return x.astype(bf16).astype(f32)


def _cmul(ar, ai, br, bi):
    return ar * br - ai * bi, ar * bi + ai * br


def _csq(ar, ai):
    t = ar * ai
    return ar * ar - ai * ai, t + t


def _csqrt(wr, wi):
    big = jnp.clip(jnp.maximum(jnp.abs(wr), jnp.abs(wi)), 2.0 ** -125, 2.0 ** 125)
    e = jnp.log2(big)
    down = jnp.exp2(-e)
    xr, xi = wr * down, wi * down
    p = jnp.exp2(0.5 * jnp.log2(xr * xr + xi * xi)) + jnp.abs(xr)
    q = jnp.exp2(0.5 * ((e - 1.0) - jnp.log2(jnp.maximum(p, 2.0 ** -60))))
    t, o = p * q, xi * q
    pos = xr >= 0
    return jnp.where(pos, t, o), jnp.where(pos, o, t)


def _pack2(a, b):
    both = jnp.concatenate([a, b], axis=1).astype(bf16).reshape(2 * a.shape[0], 128)
    return pltpu.bitcast(both, i32)


def _ln_stats(s1, s2):
    m = s1 * (1.0 / D)
    v = _rnd(jnp.maximum(s2 * (1.0 / D) - m * m, 0.0))
    return _rnd(m), 1.0 / _rnd(jnp.sqrt(_rnd(v + _rnd(jnp.full_like(v, EPS)))))


def _merge(a, b):
    v = a + b[::-1]
    if len(v) > CAP:
        v = [jnp.maximum(p, q) for p, q in zip(v[:CAP], v[CAP:])]
    n = len(v) // 2
    while n:
        v = [jnp.minimum(p, v[i - n]) if i & n else jnp.maximum(p, v[i + n])
             for i, p in enumerate(v)]
        n //= 2
    return v


def _merge_rows(v):
    for n in (4, 2, 1):
        v = _merge(v, [pltpu.roll(p, n, 0) for p in v])
    return v


def _span(start, size, align):
    return pl.ds(start if isinstance(start, int) else pl.multiple_of(start, align), size)


def _lanes(c, n=1):
    return _span(128 * n * c, 128 * n, 128 * n)


def _row(ref, k, r, rows):
    return jnp.broadcast_to(ref[k, pl.ds(r, 1), :], (rows, 128))


def _iota(shape, axis):
    return lax.broadcasted_iota(i32, shape, axis)


def _lane_sum(v):
    return jnp.broadcast_to(jnp.sum(v, axis=1, keepdims=True), v.shape)


def _main(
    x_hbm, are_hbm, aim_hbm, bre_hbm, bim_hbm, cre_hbm, cim_hbm,
    ldt_hbm, dsk_hbm, wr_hbm, wg_hbm, wu_hbm, wd_hbm,
    o_hbm,
    ldt, dsk, wrt, prm, col, pr, pi, mul, vec, xb, xs, st1, un, ur,
    vs, ss, zs, ys, rs, hs, st2, ob, nb, wg, wu, wd, we, lb,
    sem_o, sem,
):
    x_mid, x_top, x_end = [(x_hbm, xb, k) for k in (4, 5, 6)]
    gate, up, down, last = (wg_hbm, wg, 7), (wu_hbm, wu, 8), (wd_hbm, wd, 9), (wd_hbm.at[2], we, 10)

    def copy(what, *where):
        src, dst, k = what
        return pltpu.make_async_copy(src.at[where], dst.at[where], sem.at[k])

    def fetch(what, after, i, c0, width, *band):
        rows = _span(8 * i, 8, 8)
        what[1][(*band, rows, _span(c0, 128, 128))] = after.astype(bf16)
        copy(what, *band, rows, _span(c0, width, 128)).start()

    v_cp = [pltpu.make_async_copy(a, b, sem.at[0])
            for a, b in ((ldt_hbm, ldt), (dsk_hbm, dsk), (wr_hbm, wrt))]
    p_cp = {lo: [copy((src, prm.at[k], 1 + j), slice(8 * lo, 8 * hi))
                 for k, src in enumerate((are_hbm, aim_hbm, bre_hbm, bim_hbm, cre_hbm, cim_hbm))]
            for j, (lo, hi) in enumerate(zip(PARTS, PARTS[1:]))}
    x0, x1, x2 = X_ROWS
    for k, c in enumerate(sum(p_cp.values(), v_cp)
                          + [copy(x_mid, slice(x0, x1)), copy(x_top, slice(0, x0))]):
        c.start(priority=int(k > 8 or k % 2))

    lane8, sub8 = _iota((8, 128), 1), _iota((8, 128), 0)
    zero8, zero16 = jnp.zeros((8, 128), f32), jnp.zeros((16, 128), f32)
    nb[...] = jnp.zeros((L, 128), f32)
    for c in v_cp:
        c.wait()
    for k, ref in enumerate((ldt, dsk, wrt)):
        row = ref[...].astype(f32).reshape(1, D)
        row = jnp.concatenate([row, jnp.zeros((1, 640 - D), f32)], axis=1)
        for t in range(5):
            v = jnp.broadcast_to(row[:, 128 * t:128 * t + 128], (8, 128))
            vec[k, t] = v if k else _rnd(jnp.exp(v))

    def own(k, g):
        return jnp.where(lane8 - sub8 == 8 * (g & 15), vec[k, g >> 4], 0.0)

    def step_size(g):
        col[2, _span(8 * g, 8, 8), :] = _lane_sum(own(0, g))

    paced = (D - x1) // 4
    pl.loop(0, NG - paced, unroll=NG - paced)(step_size)
    vec[3, 0] = _lane_sum(sum(vec[2, t] for t in range(5)))

    zero = jnp.minimum(pltpu.bitcast(vec[1, 0], i32)[0, 0] & 1, 0)
    never = (lane8 < zero, sub8 < zero)

    def step(g, *after):
        rows = _span(8 * g, 8, 8)
        dt = col[2, rows, :]
        for mask, v in zip(never, after):
            dt = jnp.where(mask, v, dt)
        mag, ph = jnp.exp(dt * prm[0, rows, :].astype(f32)), dt * prm[1, rows, :].astype(f32)
        cos = jnp.cos(ph)
        mul[4, rows, :], mul[5, rows, :] = mag * cos, mag * jnp.sin(ph)
        return mag, cos

    def powers(g, after):
        rows = _span(8 * g, 8, 8)
        dt = jnp.where(never[0], after, col[2, rows, :])
        br, bi, cr, ci = [prm[k, rows, :].astype(f32) for k in range(2, 6)]
        w = _cmul(cr, ci, dt * br, dt * bi)
        col[0, rows, :] = _lane_sum(w[0] + own(1, g))
        col[1, rows, :] = _lane_sum(own(2, g))
        a = mul[4, rows, :], mul[5, rows, :]
        v = _csqrt(*_cmul(*w, *a))
        a = _csq(*a)
        for j in range(8):
            pr[pl.ds(j * PS + rows.start, 8), :], pi[pl.ds(j * PS + rows.start, 8), :] = v
            done, v = v[0], _cmul(*v, *a)
        for _ in range(3):
            a = _csq(*a)
        mul[0, rows, :], mul[1, rows, :] = a
        mul[2, rows, :], mul[3, rows, :] = _csq(*_csq(*a))
        return done

    def set_up(lo, hi, carry):
        def one(g, carry):
            trig, done = carry
            mag = cos = new = trig[0]
            if lo < NG:
                mag, cos = step(g, trig[0], done[0])
            if lo < paced:
                step_size(g + NG - paced)
                fetch(x_mid if 4 * lo < x2 - x1 else x_end, mag,
                      x1 // 8 + (g >> 1), L // 2 * (g & 1), L // 2)
            if lo >= 3:
                new = powers(g - 3, trig[0])
            return trig[1:] + [cos], done[1:] + [new]

        return lax.fori_loop(lo, hi, one, carry, unroll=hi - lo)

    carry = ([zero8] * 3, [zero8] * 4)
    cuts = sorted(PARTS + (3, (x2 - x1) // 4, paced, NG + 3))
    for lo, hi in zip(cuts, cuts[1:]):
        for c in p_cp.get(lo, []):
            c.wait()
        for r in range(0, DB if lo == PARTS[-2] else 0, 8):
            copy(gate, slice(None), pl.ds(r, 8), slice(GW, F)).start(priority=1)
        carry = set_up(lo, hi, carry)

    def moments(i, part, rows, after):
        s1 = s2 = jnp.concatenate([jnp.where(never[0], after, 0.0)] * 2, axis=1)
        if part:
            s1, s2 = st1[i, 0], st1[i, 1]
        for q in rows:
            v = xb[pl.ds(q, 8), _lanes(i, 2)].astype(f32)
            for e in range(2):
                xs[pl.ds((2 * i + e) * HS + q, 8), :] = v[:, 128 * e:128 * e + 128]
            s1, s2 = s1 + v, s2 + v * v
        fetch(down, v[:, :128], i >> 1, F // 3 * part, F // 3, i & 1)
        if part:
            s1, s2 = _ln_stats(*[jnp.broadcast_to(jnp.sum(v, axis=0, keepdims=True), v.shape)
                                 for v in (s1, s2)])
        st1[i, 0], st1[i, 1] = s1, s2
        return s2[:, :128]

    flip = jnp.where(_iota((128, 128), 0) == _iota((128, 128), 1) ^ 63, 1.0, 0.0).astype(bf16)

    def normalise(i):
        m, s = [[st1[i, n, :, _lanes(e)] for e in range(2)] for n in range(2)]
        for q in range(D // 16):
            xa, xc = [[xs[pl.ds(c * HS + 16 * q + 8 * e, 8), :] for e in range(2)]
                      for c in (2 * i, 2 * i + 1)]
            u = [((xa[e] - m[0]) * s[0], (xc[e] - m[1]) * s[1]) for e in range(2)]
            w = [_pack2(*v) for v in u]
            if q % 3 == 0:
                r = jnp.dot(jnp.concatenate(u[0] + u[1], axis=0).astype(bf16), flip,
                            preferred_element_type=f32)
                r = [_pack2(r[n:n + 8], r[n + 8:n + 16]) for n in (0, 16)]
            else:
                r = [jnp.take_along_axis(v, lane8 ^ 63, axis=1, mode="promise_in_bounds")
                     for v in w]
            for e in range(2):
                rows = pl.ds(i * HS + 16 * q + 8 * e, 8)
                un[rows, :], ur[rows, :] = w[e], r[e]
        fetch(down, u[0][0], i >> 1, F // 3 * 2, F // 3, i & 1)


    @pl.loop(0, 1 + zero)
    def _(_):
        for part, spans in enumerate(([(x_mid, x0, x2)], [(x_top, 0, x0), (x_end, x2, D)])):
            for what, a, b in spans:
                copy(what, slice(a, b)).wait()
            rows = [q for _, a, b in spans for q in range(a, b, 8)]
            lax.fori_loop(0, NT // 2, lambda i, v: moments(i, part, rows, v), zero8,
                          unroll=NT // 2)
        pl.loop(0, NT // 2, unroll=NT // 2)(normalise)

    left8, right8 = lane8 < 64, lane8 >= 64
    lane16, row16 = _iota((16, 128), 1), _iota((16, 128), 0)
    lane32, row32 = _iota((32, 128), 1), 2 * _iota((32, 128), 0)
    tri0, tri1 = (lane32 >= row32) & (lane32 < 64), lane32 >= row32 + 64

    def v_tile(r, k):
        return pltpu.bitcast(vs[r, pl.ds(64 * k, 64), :], bf16)

    def channel(ref, g, k, n):
        return ref[pl.ds(g * 8 + k, n, stride=HS), :]

    def vandermonde(g, r, k):
        ch = g * 8 + k
        vr, vi = pr[pl.ds(ch, 8, stride=PS), :], pi[pl.ds(ch, 8, stride=PS), :]
        odd = _cmul(vr, vi, _row(mul, 4, ch, 8), _row(mul, 5, ch, 8))
        vr, vi = jnp.concatenate([vr, odd[0]], axis=0), jnp.concatenate([vi, odd[1]], axis=0)
        mr, mi = _row(mul, 0, ch, 16), _row(mul, 1, ch, 16)
        re, im = [], []
        for q in range(4):
            re.append(_pack2(vr[:8], vr[8:]))
            im.append(_pack2(vi[:8], vi[8:]))
            vr, vi = _cmul(vr, vi, mr, mi)
        for q, v in enumerate(re + im):
            vs[r, pl.ds(64 * k + 8 * q, 8), :] = v
        return odd[0]

    def chunk_states(g, r, k):
        p1 = channel(ur, g, k, NT // 2)
        p2 = pltpu.roll(p1, 64, 1)
        lhs = jnp.concatenate([
            jnp.where(left8, p1, 0), jnp.where(right8, p2, 0),
            jnp.where(left8, p2, 0), jnp.where(right8, p1, 0)], axis=0)
        ss[pl.ds(SS * (8 * r + k), 64), :] = jnp.dot(
            pltpu.bitcast(lhs, bf16), v_tile(r, k), preferred_element_type=f32)

    def scan(g, r, k, state):
        def s_at(row):
            return ss[pl.ds(SS * 8 * r + row, 8, stride=SS), :]

        seen = []
        if k == 0:
            rows = _span(8 * g, 8, 8)
            seen.append((pr[rows, :], -pi[rows, :]))
            state = (mul[2, rows, :], mul[3, rows, :], s_at(0), -s_at(16))
        cr, ci, xr, xi = state
        for h in range(max(4 * k, 1), 4 * k + 4):
            seen.append((xr, xi))
            base = 32 * (h % 2) + h // 2
            if h < 31:
                xr, xi = ((cr * xr + s_at(base)) + ci * xi,
                          (cr * xi - s_at(base + 16)) - ci * xr)
        for e in range(2):
            for p in range(2):
                zs[r, pl.ds(16 * e + 8 * p + k, 8, stride=ZS), :] = _pack2(
                    seen[e][p], seen[2 + e][p])
        return cr, ci, xr, xi

    def read_out(r, k, y):
        o = lax.dot_general(pltpu.bitcast(zs[r, pl.ds(ZS * k, 32), :], bf16), v_tile(r, k),
                            NT_DIMS, preferred_element_type=f32)
        ys[y, pl.ds(ZS * k, 16), :] = jnp.where(lane16 < 64, o[0:16], o[48:64])
        ys[y, pl.ds(ZS * k + 16, 16), :] = jnp.where(lane16 < 64, o[32:48], o[16:32])

    def taps(g, r):
        ra, rb = pl.ds(0, 8, stride=ZS), pl.ds(16, 8, stride=ZS)
        ya, yb = ys[r, ra, :], ys[r, rb, :]
        ys[r, ra, :], ys[r, rb, :] = jnp.where(left8, 0.0, ya), jnp.where(left8, yb, 0.0)
        kk = jnp.where(left8, ya, yb)
        diag = col[0, _span(8 * g, 8, 8), :]
        ka = pltpu.roll(kk, 1, 1) + pltpu.roll(kk, 65, 1)
        kb = pltpu.roll(kk, 2, 1) + pltpu.roll(kk, 66, 1)
        pos = lane8 & 63
        rs[r] = _pack2(jnp.where(pos == 0, diag, ka),
                       jnp.where(pos == 0, 0.0, jnp.where(pos == 1, diag, kb)))

    def finish(g, r, k, older, acc):
        yq = pltpu.roll(ys[r, pl.ds(ZS * k + 16, 16), :], 64, 1)
        rb = pltpu.roll(_row(rs, r, k, 32), 0, 1, stride=2, stride_axis=0)
        t = jnp.concatenate([jnp.where(tri0, rb, 0), jnp.where(tri1, rb, 0)], axis=0)
        u = channel(un, g, k, NT // 2)
        for e in range(0 if older is None else 2):
            u = jnp.where(never[e], pltpu.bitcast(older[8 * e:8 * e + 8], i32), u)
        y = jnp.dot(pltpu.bitcast(u, bf16), pltpu.bitcast(t, bf16), preferred_element_type=f32)
        h = y + (channel(xs, g, k, NT) + (yq + ys[r, pl.ds(ZS * k, 16), :]))
        hs[pl.ds(g * 8 + k, NT, stride=HS), :] = h
        return yq, h[:8], (acc[0] + h, acc[1] + h * h, acc[2] + h * _row(col, 1, g * 8 + k, NT))

    def pace(g, k, after):
        if k == 6:
            fetch(gate, after, lax.div(g, 3), 0, GW, lax.rem(g, 3))
        elif k % 2 == 0:
            q, r = lax.div(3 * g + k // 2, RU), lax.rem(3 * g + k // 2, RU)
            fetch(up, after, r * (NG // RU) + lax.div(q, 3), F // 3 * lax.rem(q, 3), F // 3)

    def body(g0, q0, steps, carry):
        acc, rolled = carry[0], dict(zip(range(-Q_LAG, 0), carry[1]))
        state = None
        for t in range(steps):
            def at(lag):
                q, k = divmod(t - lag, 8)
                if q0 + q >= 0:
                    return g0 + q, (q0 + q) % RING, k

            if w := at(LAG_C):
                read_out(*w[1:], w[1])
            v = vandermonde(*at(0))
            if not at(LAG_D):
                pace(NG + (t - LAG_D) // 8, t % 8, v)
            if w := at(LAG_B):
                state = scan(*w, state)
            chunk_states(*at(0))
            if (w := at(LAG_K)) and w[2] == 0:
                taps(*w[:2])
            if w := at(LAG_D):
                rolled[t], h, acc = finish(*w, rolled.get(t - Q_LAG), acc)
                pace(w[0], w[2], h)
        return acc, [rolled[t] for t in range(steps - Q_LAG, steps)]

    fill, n = pl.cdiv(LAG_D + Q_LAG, 8 * RING), NG // RING

    def steady(lo, hi, carry):
        return lax.fori_loop(lo, hi, lambda j, c: body(j * RING, fill * RING, 8 * RING, c),
                             carry, unroll=hi - lo)[0]

    def first_half(acc):
        return steady(fill, n // 2, body(0, 0, 8 * RING * fill, (acc, [])))

    def second_half(acc):
        for r in range(32, DB, 8):
            copy(down, slice(0, 2), pl.ds(r, 8)).start(priority=1)
        copy(last, slice(0, DB - 8 * (11 + NQ))).start(priority=1)
        return steady(n // 2, n, (acc, [zero16] * Q_LAG))

    def drain(acc):
        def slot(g):
            return g % RING + 2 * (g >= NG - 2)

        state = None
        for ch in range(D - LAG_B, D):
            state = scan(ch // 8, ch // 8 % RING, ch % 8, state)
        for g in (NG - 5, NG - 4):
            taps(g, slot(g))
        for ch in range(D - LAG_C, D):
            read_out(ch // 8 % RING, ch % 8, slot(ch // 8))
        for ch in range(D - LAG_D, D):
            for g in range(NG - 3, NG if ch == D - 32 else 0):
                taps(g, slot(g))
            g, k = divmod(ch, 8)
            _, h, acc = finish(g, slot(g), k, None, acc)
            if k % 3 == 0:
                fetch(last, h, g - 2 * DB // 8, F // 9 * k, F // 3)
        return acc

    acc = (zero16,) * 3
    for part in (first_half, second_half, drain):
        acc = lax.fori_loop(0, 1 + zero, lambda _, c: part(c), acc)

    m2, inv2 = _ln_stats(acc[0], acc[1])
    score = (acc[2] - m2 * jnp.concatenate([vec[3, 0]] * 2)) * inv2
    st2[0], st2[1], st2[2] = m2, inv2, _rnd(score)

    bits = pltpu.bitcast(jnp.where(score == 0.0, 0.0, score), i32) >> 13
    rank = jnp.where(score != score, 0, jnp.where(bits >= 0, bits + (1 << 18), -1 - bits))
    key = pltpu.bitcast((1 << 29) + (rank << 11) + (L - 1 - (row16 * 128 + lane16)), f32)

    def write_tiles(j, after, run):
        m, s = [[_row(st2, n, 2 * j + e, 8) for e in range(2)] for n in range(2)]
        scale, shift = [v + 1.0 for v in s], [a * b for a, b in zip(m, s)]
        done = [after] * 2
        for q in range(NG):
            if q % run == 0:
                mult = [jnp.where(never[0], done[-2], v) for v in scale]
            v = [hs[pl.ds((2 * j + e) * HS + 8 * q, 8), :] * mult[e] - shift[e] for e in range(2)]
            ob[pl.ds(8 * q, 8), _lanes(j, 2)] = jnp.concatenate(v, axis=1).astype(bf16)
            if q % 24 == 0 and j < 5:
                fetch(last, v[0], DB // 8 - 7 - j, F // 72 * q, F // 3)
            if q % run == run - 1:
                done.append(v[1])
        return done[-1]

    def spread(v, shift, stride, after):
        return [jnp.where(never[1], after, pltpu.roll(p, shift, 1, stride=stride, stride_axis=0))
                for p in v]

    tops = _merge_rows(_merge([key[:8]], [key[8:]]))
    tops = _merge_rows(spread(tops, 0, 1, write_tiles(0, tops[0], 3)))
    after = write_tiles(1, tops[0], 3)
    tops = _merge_rows(_merge(spread(tops, 0, 8, after), spread(tops, 64, 8, after)))
    after = tops[0]
    for j in (2, 3, 4):
        after = write_tiles(j, after, 2)
    st2[3] = jnp.where(key >= jnp.concatenate([tops[-1]] * 2), 1.0, 0.0)
    tops = [~pltpu.bitcast(v, i32) & (L - 1) for v in tops]
    tops = [[pltpu.bitcast((1 << 29) + ((v & 127) << 11) + v, f32)] for v in tops]
    while len(tops) > 1:
        tops = [_merge(a, b) for a, b in zip(tops[::2], tops[1::2])]
    idx = [pltpu.bitcast(v, i32)[0, 0] & (L - 1) for v in tops[0]]

    tile, lane = [v >> 7 for v in idx], [v & 127 for v in idx]
    turn, turns = [0, 0], 0
    for j in range(2, CAP):
        turn.append(jnp.where(lane[j] == lane[j - 2], turn[j - 2] + 1, 0))
        turns = jnp.maximum(turns, turn[j] + 1)

    def gather(n):
        at = [jnp.where(turn[j] == n, lane[j], -1) for j in range(CAP)]
        rows = []
        for team in (range(0, CAP, 2), range(1, CAP, 2)):
            onehot, merged = zero8, []
            for j in team:
                onehot = jnp.where((sub8 == j) & (lane8 == at[j]), 1.0, onehot)
            for q in range(0, D, 16):
                v = hs[pl.ds(tile[team[0]] * HS + q, 16), :]
                for j in team[1:]:
                    v = jnp.where(lane16 == at[j], hs[pl.ds(tile[j] * HS + q, 16), :], v)
                merged.append(v)
            merged = jnp.concatenate(merged + merged[-4:], axis=0).astype(bf16)
            rows.append(lax.dot_general(onehot.astype(bf16), merged, NT_DIMS,
                                        preferred_element_type=f32))
        stat = [zero8] * 3
        for j in range(CAP):
            pick = (sub8 == j) & (lane8 == at[j])
            stat = [jnp.where(pick, _row(st2, k, tile[j], 8), v) for k, v in enumerate(stat)]
        return [rows[0] + rows[1]] + [_lane_sum(v) for v in stat]

    hsel, m_j, s_j, r_j = lax.fori_loop(
        1, turns, lambda n, c: [a + b for a, b in zip(c, gather(n))], gather(0))
    xsel = _rnd(_rnd(hsel - jnp.tile(m_j, (1, 5))) * jnp.tile(s_j, (1, 5)))

    x_main = xsel[:, :512].astype(bf16)
    x_tail = jnp.concatenate([xsel[:, 512:]] * 2, axis=0)
    x_tail = jnp.where((row16 < 8) == (lane16 < 64), x_tail, 0.0).astype(bf16)
    for c in (copy(gate, slice(None)), copy(up, slice(None)), copy(down, slice(0, 2))):
        c.wait()

    late, fresh = 0, []
    for j in range(CAP):
        fresh.append(((late >> tile[j]) & 1) == 0)
        late = late | (1 << tile[j])

    def bands(ref, cols):
        v = ref[:, :, cols]
        return v.reshape(-1, v.shape[2])

    acts, w_t = [], []

    def transpose_ahead(v):
        b, t = divmod(len(w_t), F // 128)
        if b == 3:
            return v
        w_t.append(pltpu.bitcast(bands(wd, _lanes(t))[128 * b:128 * b + 128].T, i32))
        return jnp.where(never[t % 2], pltpu.bitcast(w_t[-1][56:], v.dtype) + v, v)

    popped, sent = [xsel[:, :128]] * 2, 0
    for k in range(F // FW):
        f = pl.ds(k * FW, FW)
        x_k = pltpu.bitcast(x_tail, i32)
        for _ in range(TR[k]):
            x_k = transpose_ahead(x_k)
        if k in WT:
            x_k = jnp.where(never[1], pltpu.bitcast(write_tiles(WT[k], popped[-2], 1), i32), x_k)
            for c in range(sent, sent := 2 * WT[k] + 2):
                pl.when(((late >> c) & 1) == 0)(lambda: pltpu.make_async_copy(
                    ob.at[:, _lanes(c)], o_hbm.at[:, _lanes(c)], sem_o).start(priority=c % 2))
        tail = jnp.concatenate([bands(wg, f)[512:], wu[pl.ds(512, 64), f]], axis=0)
        tail = jnp.dot(pltpu.bitcast(x_k, bf16), tail, preferred_element_type=f32)
        a = jnp.dot(x_main, bands(wg, f)[:512], preferred_element_type=f32)
        b = jnp.dot(x_main, wu[pl.ds(0, 512), f], preferred_element_type=f32)
        popped.append(tail[:8, :128])
        for e, v in enumerate((tail, a, b) if k < NQ else ()):
            fetch(last, v[:8, :128], DB // 8 - 12 - k, F // 3 * e, F // 3)
        a, b = _rnd(a + tail[:8]), _rnd(b + tail[8:])
        act = _rnd(a * jax.nn.sigmoid(a)) * b
        acts += [act[:, n:n + 128] for n in range(0, FW, 128)]
    weight = _rnd(jax.nn.sigmoid(r_j))
    routed = [_row(st2, 3, v, 8) > 0 for v in tile]

    def project(d0, ties):
        nd = min(128, D - d0)
        y = jnp.zeros((8, nd), f32)
        for t, act in enumerate(acts):
            if d0 or t >= TN:
                act = transpose_ahead(act)
            if t in ties:
                act = jnp.where(never[0], ties[t], act)
            if d0 < 2 * DB:
                y = y + jnp.dot(act.astype(bf16), pltpu.bitcast(w_t[d0 // 128 * len(acts) + t], bf16),
                                preferred_element_type=f32)
            else:
                y = y + lax.dot_general(act.astype(bf16), we[pl.ds(d0 - 2 * DB, nd), _lanes(t)],
                                        NT_DIMS, preferred_element_type=f32)
        return y

    def patch(d0, y):
        nd = y.shape[1]
        rows = pl.ds(d0, nd)
        new = hsel[:, d0:d0 + nd] + _rnd(xsel[:, d0:d0 + nd] + _rnd(_rnd(y) * weight[:, :nd]))
        if nd < 128:
            new = jnp.concatenate([new, zero8[:, nd:]], axis=1)
        for j in range(CAP):
            nb[pl.ds(idx[j], 1), :] = new[j:j + 1]
        for j in range(CAP):
            cols = _lanes(tile[j])
            one = pltpu.bitcast(nb[cols, :].astype(bf16).T[:nd], i32)
            for q in range(0, nd, 16):
                lb[j][pl.ds(d0 + q, 16), :] = pltpu.bitcast(jnp.where(
                    routed[j], one[q // 2:q // 2 + 8],
                    pltpu.bitcast(ob[pl.ds(d0 + q, 16), cols], i32)), bf16)
        for j in range(CAP):
            pl.when(fresh[j])(lambda: pltpu.make_async_copy(
                lb[j].at[rows], o_hbm.at[rows, _lanes(tile[j])], sem_o).start(priority=j % 2))
        return new, pltpu.bitcast(one[-8:], f32)

    begun, ended = patch(0, project(0, {}))
    held = project(128, {19: begun}), project(256, {32: ended})
    copy(last, slice(None)).wait()
    ended = patch(128, held[0])[1], patch(256, held[1])[1]
    begun = patch(384, project(384, dict(zip(TIE, ended))))[0]
    patch(512, project(512, {19: begun}))


def _kernel(*refs):
    pl.run_scoped(lambda sem: _main(*refs, sem), pltpu.SemaphoreType.DMA((11,)))
    pltpu.make_async_copy(refs[13], refs[13], refs[-1]).wait()


@jax.jit
def pallas_sequential_preLN__ssm_conv_s4__moe_arch_mod__prompt_kernel(
    A_u: jax.Array,
    A_A_re: jax.Array,
    A_A_im: jax.Array,
    A_B_re: jax.Array,
    A_B_im: jax.Array,
    A_C_re: jax.Array,
    A_C_im: jax.Array,
    A_log_dt: jax.Array,
    A_Dskip: jax.Array,
    B_x: jax.Array,
    B_w_r: jax.Array,
    B_w_gate: jax.Array,
    B_w_up: jax.Array,
    B_w_down: jax.Array,
):
    del B_x
    hbm = pl.BlockSpec(memory_space=pltpu.HBM)
    out = pl.pallas_call(
        _kernel,
        out_shape=jax.ShapeDtypeStruct((D, L), bf16),
        in_specs=[hbm] * 13,
        out_specs=hbm,
        scratch_shapes=[
            pltpu.VMEM((D,), bf16),
            pltpu.VMEM((D,), bf16),
            pltpu.VMEM((D,), bf16),
            pltpu.VMEM((6, D, N), bf16),
            pltpu.VMEM((3, D, 128), f32),
            pltpu.VMEM((9 * 584, N), f32),
            pltpu.VMEM((9 * 584, N), f32),
            pltpu.VMEM((6, D, N), f32),
            pltpu.VMEM((4, 5, 8, 128), f32),
            pltpu.VMEM((D, L), bf16),
            pltpu.VMEM((17 * 584, 128), f32),
            pltpu.VMEM((NT // 2, 2, 8, 256), f32),
            pltpu.VMEM((9 * 584, 128), i32),
            pltpu.VMEM((9 * 584, 128), i32),
            pltpu.VMEM((RING, 512, N), i32),
            pltpu.VMEM((RING * 8 * SS + 72, N), f32),
            pltpu.VMEM((RING, 8 * ZS + 40, N), i32),
            pltpu.VMEM((RING + 2, 8 * ZS + 40, 128), f32),
            pltpu.VMEM((RING + 2, 8, 128), i32),
            pltpu.VMEM((17 * 584, 128), f32),
            pltpu.VMEM((4, NT, 128), f32),
            pltpu.VMEM((D, L), bf16),
            pltpu.VMEM((L, 128), f32),
            pltpu.VMEM((3, DB, F), bf16),
            pltpu.VMEM((D, F), bf16),
            pltpu.VMEM((2, DB, F), bf16),
            pltpu.VMEM((DB, F), bf16),
            [pltpu.VMEM((D, 128), bf16)] * CAP,
            pltpu.SemaphoreType.DMA(()),
        ],
        compiler_params=pltpu.CompilerParams(
            vmem_limit_bytes=100 * 1024 * 1024,
            flags={"XLA_TPU_FORCE_LP_LLO_SCHEDULER": True},
        ),
    )(
        A_u.reshape(L, D).T, A_A_re, A_A_im, A_B_re, A_B_im, A_C_re, A_C_im,
        A_log_dt, A_Dskip, B_w_r, B_w_gate.reshape(3, DB, F), B_w_up,
        B_w_down.T.reshape(3, DB, F),
    )
    return out.T.reshape(1, L, D)
```

```python
import jax
import jax.numpy as jnp
from jax import lax
import jax.experimental.pallas as pl
import jax.experimental.pallas.tpu as pltpu

D = 576
L = 2048
N = 128
F = 4608
CAP = 8
EPS = 1e-5

NT = L // 128
NG = D // 8
DB = D // 3

HS = 580
PS = 577
SS = 65
ZS = 36

LAG = 8
PARTS = (LAG, 20, 40, NG)
X_ROWS = (112, 312, 488)
RING = 4
LAG_B, LAG_C, LAG_K, LAG_D = 16, 24, 42, 48
Q_LAG = 4
FW = 512
GW = 1024
TR = (0, 4, 12, 12, 12, 12, 12, 12, 12)
WT = {3: 5, 4: 6, 6: 7}
NL = 14
RU = 4
TIE = (28, 35)
TN = 12
LM = 0
NF = 3
PK = 1
FS = 3

f32 = jnp.float32
bf16 = jnp.bfloat16
i32 = jnp.int32
NT_DIMS = (((1,), (1,)), ((), ()))


def _rnd(x):
    return x.astype(bf16).astype(f32)


def _cmul(ar, ai, br, bi):
    return ar * br - ai * bi, ar * bi + ai * br


def _csq(ar, ai):
    t = ar * ai
    return ar * ar - ai * ai, t + t


def _csqrt(wr, wi):
    big = jnp.clip(jnp.maximum(jnp.abs(wr), jnp.abs(wi)), 2.0 ** -125, 2.0 ** 125)
    e = jnp.log2(big)
    down = jnp.exp2(-e)
    xr, xi = wr * down, wi * down
    p = jnp.exp2(0.5 * jnp.log2(xr * xr + xi * xi)) + jnp.abs(xr)
    q = jnp.exp2(0.5 * ((e - 1.0) - jnp.log2(jnp.maximum(p, 2.0 ** -60))))
    t, o = p * q, xi * q
    pos = xr >= 0
    return jnp.where(pos, t, o), jnp.where(pos, o, t)


def _pack2(a, b):
    both = jnp.concatenate([a, b], axis=1).astype(bf16).reshape(2 * a.shape[0], 128)
    return pltpu.bitcast(both, i32)


def _ln_stats(s1, s2):
    m = s1 * (1.0 / D)
    v = _rnd(jnp.maximum(s2 * (1.0 / D) - m * m, 0.0))
    return _rnd(m), 1.0 / _rnd(jnp.sqrt(_rnd(v + _rnd(jnp.full_like(v, EPS)))))


def _merge(a, b):
    v = a + b[::-1]
    if len(v) > CAP:
        v = [jnp.maximum(p, q) for p, q in zip(v[:CAP], v[CAP:])]
    n = len(v) // 2
    while n:
        v = [jnp.minimum(p, v[i - n]) if i & n else jnp.maximum(p, v[i + n])
             for i, p in enumerate(v)]
        n //= 2
    return v


def _merge_rows(v):
    for n in (4, 2, 1):
        v = _merge(v, [pltpu.roll(p, n, 0) for p in v])
    return v


def _span(start, size, align):
    return pl.ds(start if isinstance(start, int) else pl.multiple_of(start, align), size)


def _lanes(c, n=1):
    return _span(128 * n * c, 128 * n, 128 * n)


def _row(ref, k, r, rows):
    return jnp.broadcast_to(ref[k, pl.ds(r, 1), :], (rows, 128))


def _iota(shape, axis):
    return lax.broadcasted_iota(i32, shape, axis)


def _lane_sum(v):
    return jnp.broadcast_to(jnp.sum(v, axis=1, keepdims=True), v.shape)


def _main(
    x_hbm, are_hbm, aim_hbm, bre_hbm, bim_hbm, cre_hbm, cim_hbm,
    ldt_hbm, dsk_hbm, wr_hbm, wg_hbm, wu_hbm, wd_hbm,
    o_hbm,
    ldt, dsk, wrt, prm, col, pr, pi, mul, vec, xb, xs, st1, un, ur,
    vs, ss, zs, ys, rs, hs, st2, ob, nb, wg, wu, wd, we, lb,
    sem_o, sem,
):
    x_mid, x_top, x_end = [(x_hbm, xb, k) for k in (4, 5, 6)]
    gate, up, down, last = (wg_hbm, wg, 7), (wu_hbm, wu, 8), (wd_hbm, wd, 9), (wd_hbm.at[2], we, 10)

    def copy(what, *where):
        src, dst, k = what
        return pltpu.make_async_copy(src.at[where], dst.at[where], sem.at[k])

    def fetch(what, after, i, c0, width, *band):
        rows = _span(8 * i, 8, 8)
        what[1][(*band, rows, _span(c0, 128, 128))] = after.astype(bf16)
        copy(what, *band, rows, _span(c0, width, 128)).start()

    def queue(what, m):
        bands, c0 = (3, GW) if what is gate else (2, 0)
        width = (F - c0) // 4
        copy(what, slice(0, bands), _span(8 * (m >> 2), 8, 8),
             _span(c0 + width * (m & 3), width, 128)).start(priority=1)

    v_cp = [pltpu.make_async_copy(a, b, sem.at[0])
            for a, b in ((ldt_hbm, ldt), (dsk_hbm, dsk), (wr_hbm, wrt))]
    v_cp += [copy((src, prm.at[k], 0), slice(0, 8 * PARTS[0]))
             for k, src in enumerate((are_hbm, aim_hbm))]
    p_cp = {lo: [copy((src, prm.at[k], 1 + j), slice(8 * (lo - LAG * (k > 1)),
                                                      8 * (hi - LAG * (k > 1 and hi < NG))))
                 for k, src in enumerate((are_hbm, aim_hbm, bre_hbm, bim_hbm, cre_hbm, cim_hbm))]
            for j, (lo, hi) in enumerate(zip(PARTS, PARTS[1:]))}
    x0, x1, x2 = X_ROWS
    for k, c in enumerate(sum(p_cp.values(), v_cp)
                          + [copy(x_mid, slice(x0, x1)), copy(x_top, slice(0, x0))]):
        c.start(priority=int(k > 10 or (k > 4 and k % 2)))

    lane8, sub8 = _iota((8, 128), 1), _iota((8, 128), 0)
    zero8, zero16 = jnp.zeros((8, 128), f32), jnp.zeros((16, 128), f32)
    nb[...] = jnp.zeros((L, 128), f32)
    for c in v_cp:
        c.wait()
    for k, ref in enumerate((ldt, dsk, wrt)):
        row = ref[...].astype(f32).reshape(1, D)
        row = jnp.concatenate([row, jnp.zeros((1, 640 - D), f32)], axis=1)
        for t in range(5):
            v = jnp.broadcast_to(row[:, 128 * t:128 * t + 128], (8, 128))
            vec[k, t] = v if k else _rnd(jnp.exp(v))

    def own(k, g):
        return jnp.where(lane8 - sub8 == 8 * (g & 15), vec[k, g >> 4], 0.0)

    def step_size(g):
        col[2, _span(8 * g, 8, 8), :] = _lane_sum(own(0, g))

    paced = (D - x1) // 4
    pl.loop(0, NG - paced, unroll=NG - paced)(step_size)
    vec[3, 0] = _lane_sum(sum(vec[2, t] for t in range(5)))

    zero = jnp.minimum(pltpu.bitcast(vec[1, 0], i32)[0, 0] & 1, 0)
    never = (lane8 < zero, sub8 < zero)

    def step(g, *after):
        rows = _span(8 * g, 8, 8)
        dt = col[2, rows, :]
        for mask, v in zip(never, after):
            dt = jnp.where(mask, v, dt)
        mag, ph = jnp.exp(dt * prm[0, rows, :].astype(f32)), dt * prm[1, rows, :].astype(f32)
        cos = jnp.cos(ph)
        mul[4, rows, :], mul[5, rows, :] = mag * cos, mag * jnp.sin(ph)
        return mag, cos

    def powers(g, after):
        rows = _span(8 * g, 8, 8)
        dt = jnp.where(never[0], after, col[2, rows, :])
        br, bi, cr, ci = [prm[k, rows, :].astype(f32) for k in range(2, 6)]
        w = _cmul(cr, ci, dt * br, dt * bi)
        col[0, rows, :] = _lane_sum(w[0] + own(1, g))
        col[1, rows, :] = _lane_sum(own(2, g))
        a = mul[4, rows, :], mul[5, rows, :]
        v = _csqrt(*_cmul(*w, *a))
        a = _csq(*a)
        for j in range(8):
            pr[pl.ds(j * PS + rows.start, 8), :], pi[pl.ds(j * PS + rows.start, 8), :] = v
            done, v = v[0], _cmul(*v, *a)
        for _ in range(3):
            a = _csq(*a)
        mul[0, rows, :], mul[1, rows, :] = a
        mul[2, rows, :], mul[3, rows, :] = _csq(*_csq(*a))
        return done

    def set_up(lo, hi, carry):
        def one(g, carry):
            trig, done = carry
            mag = cos = new = trig[0]
            if lo < NG:
                mag, cos = step(g, trig[0], done[0])
            if lo < paced:
                step_size(g + NG - paced)
                fetch(x_mid if 4 * lo < x2 - x1 else x_end, mag,
                      x1 // 8 + (g >> 1), L // 2 * (g & 1), L // 2)
            if lo >= LAG:
                new = powers(g - LAG, trig[0])
            return trig[1:] + [cos], done[1:] + [new]

        return lax.fori_loop(lo, hi, one, carry, unroll=hi - lo)

    carry = ([zero8] * 3, [zero8] * 4)
    cuts = sorted(set(PARTS + (0, (x2 - x1) // 4, paced, NG + LAG)))
    for lo, hi in zip(cuts, cuts[1:]):
        for c in p_cp.get(lo, []):
            c.wait()
        for m in range(24 if lo == PARTS[-2] else 0):
            queue(gate, m)
        carry = set_up(lo, hi, carry)

    def moments(i, part, rows, after):
        s1 = s2 = jnp.concatenate([jnp.where(never[0], after, 0.0)] * 2, axis=1)
        if part:
            s1, s2 = st1[i, 0], st1[i, 1]
        for q in rows:
            v = xb[pl.ds(q, 8), _lanes(i, 2)].astype(f32)
            for e in range(2):
                xs[pl.ds((2 * i + e) * HS + q, 8), :] = v[:, 128 * e:128 * e + 128]
            s1, s2 = s1 + v, s2 + v * v
            if q == 0:
                fetch(down, s1[:, :128], i >> 1, F // 3 * 2, F // 3, i & 1)
        fetch(down, v[:, :128], i >> 1, F // 3 * part, F // 3, i & 1)
        if part:
            s1, s2 = _ln_stats(*[jnp.broadcast_to(jnp.sum(v, axis=0, keepdims=True), v.shape)
                                 for v in (s1, s2)])
        st1[i, 0], st1[i, 1] = s1, s2
        return s2[:, :128]

    flip = jnp.where(_iota((128, 128), 0) == _iota((128, 128), 1) ^ 63, 1.0, 0.0).astype(bf16)

    def normalise(i):
        m, s = [[st1[i, n, :, _lanes(e)] for e in range(2)] for n in range(2)]
        for q in range(D // 16):
            xa, xc = [[xs[pl.ds(c * HS + 16 * q + 8 * e, 8), :] for e in range(2)]
                      for c in (2 * i, 2 * i + 1)]
            u = [((xa[e] - m[0]) * s[0], (xc[e] - m[1]) * s[1]) for e in range(2)]
            w = [_pack2(*v) for v in u]
            if q % NF == 0:
                r = jnp.dot(jnp.concatenate(u[0] + u[1], axis=0).astype(bf16), flip,
                            preferred_element_type=f32)
                r = [_pack2(r[n:n + 8], r[n + 8:n + 16]) for n in (0, 16)]
            else:
                r = [jnp.take_along_axis(v, lane8 ^ 63, axis=1, mode="promise_in_bounds")
                     for v in w]
            for e in range(2):
                rows = pl.ds(i * HS + 16 * q + 8 * e, 8)
                un[rows, :], ur[rows, :] = w[e], r[e]


    @pl.loop(0, 1 + zero)
    def _(_):
        for part, spans in enumerate(([(x_mid, x0, x2)], [(x_top, 0, x0), (x_end, x2, D)])):
            for what, a, b in spans:
                copy(what, slice(a, b)).wait()
            rows = [q for _, a, b in spans for q in range(a, b, 8)]
            lax.fori_loop(0, NT // 2, lambda i, v: moments(i, part, rows, v), zero8,
                          unroll=NT // 2)
        pl.loop(0, NT // 2 - LM, unroll=NT // 2 - LM)(normalise)

    left8, right8 = lane8 < 64, lane8 >= 64
    lane16, row16 = _iota((16, 128), 1), _iota((16, 128), 0)
    lane32, row32 = _iota((32, 128), 1), 2 * _iota((32, 128), 0)
    tri0, tri1 = (lane32 >= row32) & (lane32 < 64), lane32 >= row32 + 64

    def v_tile(r, k):
        return pltpu.bitcast(vs[r, pl.ds(64 * k, 64), :], bf16)

    def channel(ref, g, k, n):
        return ref[pl.ds(g * 8 + k, n, stride=HS), :]

    def vandermonde(g, r, k):
        ch = g * 8 + k
        vr, vi = pr[pl.ds(ch, 8, stride=PS), :], pi[pl.ds(ch, 8, stride=PS), :]
        odd = _cmul(vr, vi, _row(mul, 4, ch, 8), _row(mul, 5, ch, 8))
        vr, vi = jnp.concatenate([vr, odd[0]], axis=0), jnp.concatenate([vi, odd[1]], axis=0)
        mr, mi = _row(mul, 0, ch, 16), _row(mul, 1, ch, 16)
        re, im = [], []
        for q in range(4):
            re.append(_pack2(vr[:8], vr[8:]))
            im.append(_pack2(vi[:8], vi[8:]))
            vr, vi = _cmul(vr, vi, mr, mi)
        for q, v in enumerate(re + im):
            vs[r, pl.ds(64 * k + 8 * q, 8), :] = v
        return odd[0]

    def chunk_states(g, r, k):
        p1 = channel(ur, g, k, NT // 2)
        p2 = pltpu.roll(p1, 64, 1)
        lhs = jnp.concatenate([
            jnp.where(left8, p1, 0), jnp.where(right8, p2, 0),
            jnp.where(left8, p2, 0), jnp.where(right8, p1, 0)], axis=0)
        ss[pl.ds(SS * (8 * r + k), 64), :] = jnp.dot(
            pltpu.bitcast(lhs, bf16), v_tile(r, k), preferred_element_type=f32)

    def scan(g, r, k, state):
        def s_at(row):
            return ss[pl.ds(SS * 8 * r + row, 8, stride=SS), :]

        seen = []
        if k == 0:
            rows = _span(8 * g, 8, 8)
            seen.append((pr[rows, :], -pi[rows, :]))
            state = (mul[2, rows, :], mul[3, rows, :], s_at(0), -s_at(16))
        cr, ci, xr, xi = state
        for h in range(max(4 * k, 1), 4 * k + 4):
            seen.append((xr, xi))
            base = 32 * (h % 2) + h // 2
            if h < 31:
                xr, xi = ((cr * xr + s_at(base)) + ci * xi,
                          (cr * xi - s_at(base + 16)) - ci * xr)
        for e in range(2):
            for p in range(2):
                zs[r, pl.ds(16 * e + 8 * p + k, 8, stride=ZS), :] = _pack2(
                    seen[e][p], seen[2 + e][p])
        return cr, ci, xr, xi

    def read_out(r, k, y):
        o = lax.dot_general(pltpu.bitcast(zs[r, pl.ds(ZS * k, 32), :], bf16), v_tile(r, k),
                            NT_DIMS, preferred_element_type=f32)
        ys[y, pl.ds(ZS * k, 16), :] = jnp.where(lane16 < 64, o[0:16], o[48:64])
        ys[y, pl.ds(ZS * k + 16, 16), :] = jnp.where(lane16 < 64, o[32:48], o[16:32])

    def taps(g, r):
        ra, rb = pl.ds(0, 8, stride=ZS), pl.ds(16, 8, stride=ZS)
        ya, yb = ys[r, ra, :], ys[r, rb, :]
        ys[r, ra, :], ys[r, rb, :] = jnp.where(left8, 0.0, ya), jnp.where(left8, yb, 0.0)
        kk = jnp.where(left8, ya, yb)
        diag = col[0, _span(8 * g, 8, 8), :]
        ka = pltpu.roll(kk, 1, 1) + pltpu.roll(kk, 65, 1)
        kb = pltpu.roll(kk, 2, 1) + pltpu.roll(kk, 66, 1)
        pos = lane8 & 63
        rs[r] = _pack2(jnp.where(pos == 0, diag, ka),
                       jnp.where(pos == 0, 0.0, jnp.where(pos == 1, diag, kb)))

    def finish(g, r, k, older, acc):
        yq = pltpu.roll(ys[r, pl.ds(ZS * k + 16, 16), :], 64, 1)
        rb = pltpu.roll(_row(rs, r, k, 32), 0, 1, stride=2, stride_axis=0)
        t = jnp.concatenate([jnp.where(tri0, rb, 0), jnp.where(tri1, rb, 0)], axis=0)
        u = channel(un, g, k, NT // 2)
        for e in range(0 if older is None else 2):
            u = jnp.where(never[e], pltpu.bitcast(older[8 * e:8 * e + 8], i32), u)
        y = jnp.dot(pltpu.bitcast(u, bf16), pltpu.bitcast(t, bf16), preferred_element_type=f32)
        h = y + (channel(xs, g, k, NT) + (yq + ys[r, pl.ds(ZS * k, 16), :]))
        hs[pl.ds(g * 8 + k, NT, stride=HS), :] = h
        return yq, h[:8], (acc[0] + h, acc[1] + h * h, acc[2] + h * _row(col, 1, g * 8 + k, NT))

    def pace(g, k, after):
        if k == 6 + PK:
            fetch(gate, after, lax.div(g, 3), 0, GW, lax.rem(g, 3))
        elif k % 2 == PK:
            q, r = lax.div(3 * g + k // 2, RU), lax.rem(3 * g + k // 2, RU)
            fetch(up, after, r * (NG // RU) + lax.div(q, 3), F // 3 * lax.rem(q, 3), F // 3)

    def body(what, g0, q0, steps, carry):
        acc, rolled = carry[0], dict(zip(range(-Q_LAG, 0), carry[1]))
        state = None
        for t in range(steps):
            def at(lag):
                q, k = divmod(t - lag, 8)
                if q0 + q >= 0:
                    return g0 + q, (q0 + q) % RING, k

            if w := at(LAG_C):
                read_out(*w[1:], w[1])
            pace(g0 + t // 8, t % 8, vandermonde(*at(0)))
            if t % 4 == 0:
                queue(what, 24 + 2 * g0 + t // 4 - (NG if what is down else 0))
            if w := at(LAG_B):
                state = scan(*w, state)
            chunk_states(*at(0))
            if (w := at(LAG_K)) and w[2] == 0:
                taps(*w[:2])
            if w := at(LAG_D):
                rolled[t], _, acc = finish(*w, rolled.get(t - Q_LAG), acc)
        return acc, [rolled[t] for t in range(steps - Q_LAG, steps)]

    fill, n = pl.cdiv(LAG_D + Q_LAG, 8 * RING), NG // RING

    def steady(what, lo, hi, carry):
        return lax.fori_loop(lo, hi, lambda j, c: body(what, j * RING, fill * RING, 8 * RING, c),
                             carry, unroll=hi - lo)[0]

    spare = list(range(3 * NL))

    def fetch_last(after):
        r, c = divmod(spare.pop(), 3)
        fetch(last, after, DB // 8 - NL + r, F // 3 * c, F // 3)

    def first_half(acc):
        for i in range(NT // 2 - LM, NT // 2):
            normalise(i)
        return steady(gate, fill, n // 2, body(gate, 0, 0, 8 * RING * fill, (acc, [])))

    def second_half(acc):
        for m in range(16, 24):
            queue(down, m)
        return steady(down, n // 2, n, (acc, [zero16] * Q_LAG))

    def drain(acc):
        def slot(g):
            return g % RING + 2 * (g >= NG - 2)

        copy(last, slice(0, DB - 8 * NL)).start(priority=1)
        state = None
        for ch in range(D - LAG_B, D):
            state = scan(ch // 8, ch // 8 % RING, ch % 8, state)
            if ch < D - 8 and ch % 2 == 0:
                fetch_last(state[2])
        for g in (NG - 5, NG - 4):
            taps(g, slot(g))
        for ch in range(D - LAG_C, D):
            read_out(ch // 8 % RING, ch % 8, slot(ch // 8))
            if ch % 4 == 0 and ch > D - LAG_C:
                fetch_last(ys[slot(ch // 8), pl.ds(ZS * (ch % 8), 8), :])
        for ch in range(D - LAG_D, D):
            for g in range(NG - 3, NG if ch == D - 32 else 0):
                taps(g, slot(g))
            g, k = divmod(ch, 8)
            _, h, acc = finish(g, slot(g), k, None, acc)
            if ch % 6 == 5:
                fetch_last(h)
        return acc

    acc = (zero16,) * 3
    for part in (first_half, second_half, drain):
        acc = lax.fori_loop(0, 1 + zero, lambda _, c: part(c), acc)

    m2, inv2 = _ln_stats(acc[0], acc[1])
    score = (acc[2] - m2 * jnp.concatenate([vec[3, 0]] * 2)) * inv2
    st2[0], st2[1], st2[2] = m2, inv2, _rnd(score)

    bits = pltpu.bitcast(jnp.where(score == 0.0, 0.0, score), i32) >> 13
    rank = jnp.where(score != score, 0, jnp.where(bits >= 0, bits + (1 << 18), -1 - bits))
    key = pltpu.bitcast((1 << 29) + (rank << 11) + (L - 1 - (row16 * 128 + lane16)), f32)

    def write_tiles(j, after, run):
        m, s = [[_row(st2, n, 2 * j + e, 8) for e in range(2)] for n in range(2)]
        scale, shift = [v + 1.0 for v in s], [a * b for a, b in zip(m, s)]

        def some(i, done):
            mult = [jnp.where(never[0], done[0], v) for v in scale]
            for q in range(run):
                rows = _span(8 * (run * i + q), 8, 8)
                v = [hs[pl.ds((2 * j + e) * HS + rows.start, 8), :] * mult[e] - shift[e]
                     for e in range(2)]
                ob[rows, _lanes(j, 2)] = jnp.concatenate(v, axis=1).astype(bf16)
            return done[1], v[1]

        done = after, after
        for lo, hi in ((0, 12), (12, 48), (48, NG)):
            if lo and j < 5:
                fetch_last(done[1])
            done = lax.fori_loop(lo // run, hi // run, some, done, unroll=(hi - lo) // run)
        return done[1]

    def spread(v, shift, stride, after):
        return [jnp.where(never[1], after, pltpu.roll(p, shift, 1, stride=stride, stride_axis=0))
                for p in v]

    tops = _merge_rows(_merge([key[:8]], [key[8:]]))
    tops = _merge_rows(spread(tops, 0, 1, write_tiles(0, tops[0], 3)))
    after = write_tiles(1, tops[0], 3)
    tops = _merge_rows(_merge(spread(tops, 0, 8, after), spread(tops, 64, 8, after)))
    after = tops[0]
    for j in (2, 3, 4):
        after = write_tiles(j, after, 2)
    st2[3] = jnp.where(key >= jnp.concatenate([tops[-1]] * 2), 1.0, 0.0)
    tops = [~pltpu.bitcast(v, i32) & (L - 1) for v in tops]
    tops = [[pltpu.bitcast((1 << 29) + ((v & 127) << 11) + v, f32)] for v in tops]
    while len(tops) > 1:
        tops = [_merge(a, b) for a, b in zip(tops[::2], tops[1::2])]
    idx = [pltpu.bitcast(v, i32)[0, 0] & (L - 1) for v in tops[0]]

    tile, lane = [v >> 7 for v in idx], [v & 127 for v in idx]
    turn, turns = [0, 0], 0
    for j in range(2, CAP):
        turn.append(jnp.where(lane[j] == lane[j - 2], turn[j - 2] + 1, 0))
        turns = jnp.maximum(turns, turn[j] + 1)

    def gather(n):
        at = [jnp.where(turn[j] == n, lane[j], -1) for j in range(CAP)]
        rows = []
        for team in (range(0, CAP, 2), range(1, CAP, 2)):
            onehot, merged = zero8, []
            for j in team:
                onehot = jnp.where((sub8 == j) & (lane8 == at[j]), 1.0, onehot)
            for q in range(0, D, 16):
                v = hs[pl.ds(tile[team[0]] * HS + q, 16), :]
                for j in team[1:]:
                    v = jnp.where(lane16 == at[j], hs[pl.ds(tile[j] * HS + q, 16), :], v)
                merged.append(v)
            merged = jnp.concatenate(merged + merged[-4:], axis=0).astype(bf16)
            rows.append(lax.dot_general(onehot.astype(bf16), merged, NT_DIMS,
                                        preferred_element_type=f32))
        stat = [zero8] * 3
        for j in range(CAP):
            pick = (sub8 == j) & (lane8 == at[j])
            stat = [jnp.where(pick, _row(st2, k, tile[j], 8), v) for k, v in enumerate(stat)]
        return [rows[0] + rows[1]] + [_lane_sum(v) for v in stat]

    hsel, m_j, s_j, r_j = lax.fori_loop(
        1, turns, lambda n, c: [a + b for a, b in zip(c, gather(n))], gather(0))
    xsel = _rnd(_rnd(hsel - jnp.tile(m_j, (1, 5))) * jnp.tile(s_j, (1, 5)))

    x_main = xsel[:, :512].astype(bf16)
    x_tail = jnp.concatenate([xsel[:, 512:]] * 2, axis=0)
    x_tail = jnp.where((row16 < 8) == (lane16 < 64), x_tail, 0.0).astype(bf16)
    for v in (m_j, xsel[:, :128]):
        fetch_last(v)
    for c in (copy(gate, slice(None)), copy(up, slice(None)), copy(down, slice(0, 2))):
        c.wait()
    for v in (m_j, m_j):
        fetch_last(v)

    late, fresh = 0, []
    for j in range(CAP):
        fresh.append(((late >> tile[j]) & 1) == 0)
        late = late | (1 << tile[j])

    def bands(ref, cols):
        v = ref[:, :, cols]
        return v.reshape(-1, v.shape[2])

    acts, w_t = [], []

    def transpose_ahead(v):
        b, t = divmod(len(w_t), F // 128)
        if b == 3:
            return v
        w_t.append(pltpu.bitcast(bands(wd, _lanes(t))[128 * b:128 * b + 128].T, i32))
        if t % FS == 0 and spare:
            fetch_last(pltpu.bitcast(w_t[-1][:8], f32))
        return jnp.where(never[t % 2], pltpu.bitcast(w_t[-1][56:], v.dtype) + v, v)

    popped, sent = [xsel[:, :128]] * 2, 0
    for k in range(F // FW):
        f = pl.ds(k * FW, FW)
        x_k = pltpu.bitcast(x_tail, i32)
        for _ in range(TR[k]):
            x_k = transpose_ahead(x_k)
        if k in WT:
            x_k = jnp.where(never[1], pltpu.bitcast(write_tiles(WT[k], popped[-2], 1), i32), x_k)
            for c in range(sent, sent := 2 * WT[k] + 2):
                pl.when(((late >> c) & 1) == 0)(lambda: pltpu.make_async_copy(
                    ob.at[:, _lanes(c)], o_hbm.at[:, _lanes(c)], sem_o).start(priority=c % 2))
        tail = jnp.concatenate([bands(wg, f)[512:], wu[pl.ds(512, 64), f]], axis=0)
        tail = jnp.dot(pltpu.bitcast(x_k, bf16), tail, preferred_element_type=f32)
        a = jnp.dot(x_main, bands(wg, f)[:512], preferred_element_type=f32)
        b = jnp.dot(x_main, wu[pl.ds(0, 512), f], preferred_element_type=f32)
        popped.append(tail[:8, :128])
        a, b = _rnd(a + tail[:8]), _rnd(b + tail[8:])
        act = _rnd(a * jax.nn.sigmoid(a)) * b
        acts += [act[:, n:n + 128] for n in range(0, FW, 128)]
    weight = _rnd(jax.nn.sigmoid(r_j))
    routed = [_row(st2, 3, v, 8) > 0 for v in tile]

    def project(d0, ties):
        nd = min(128, D - d0)
        y = jnp.zeros((8, nd), f32)
        for t, act in enumerate(acts):
            if d0 or t >= TN:
                act = transpose_ahead(act)
            if t in ties:
                act = jnp.where(never[0], ties[t], act)
            if d0 < 2 * DB:
                y = y + jnp.dot(act.astype(bf16), pltpu.bitcast(w_t[d0 // 128 * len(acts) + t], bf16),
                                preferred_element_type=f32)
            else:
                y = y + lax.dot_general(act.astype(bf16), we[pl.ds(d0 - 2 * DB, nd), _lanes(t)],
                                        NT_DIMS, preferred_element_type=f32)
        return y

    def patch(d0, y):
        nd = y.shape[1]
        rows = pl.ds(d0, nd)
        new = hsel[:, d0:d0 + nd] + _rnd(xsel[:, d0:d0 + nd] + _rnd(_rnd(y) * weight[:, :nd]))
        if nd < 128:
            new = jnp.concatenate([new, zero8[:, nd:]], axis=1)
        for j in range(CAP):
            nb[pl.ds(idx[j], 1), :] = new[j:j + 1]
        for j in range(CAP):
            cols = _lanes(tile[j])
            one = pltpu.bitcast(nb[cols, :].astype(bf16).T[:nd], i32)
            for q in range(0, nd, 16):
                lb[j][pl.ds(d0 + q, 16), :] = pltpu.bitcast(jnp.where(
                    routed[j], one[q // 2:q // 2 + 8],
                    pltpu.bitcast(ob[pl.ds(d0 + q, 16), cols], i32)), bf16)
        for j in range(CAP):
            pl.when(fresh[j])(lambda: pltpu.make_async_copy(
                lb[j].at[rows], o_hbm.at[rows, _lanes(tile[j])], sem_o).start(priority=j % 2))
        return new, pltpu.bitcast(one[-8:], f32)

    begun, ended = patch(0, project(0, {}))
    held = project(128, {19: begun}), project(256, {32: ended})
    assert not spare
    copy(last, slice(None)).wait()
    ended = patch(128, held[0])[1], patch(256, held[1])[1]
    begun = patch(384, project(384, dict(zip(TIE, ended))))[0]
    patch(512, project(512, {19: begun}))


def _kernel(*refs):
    pl.run_scoped(lambda sem: _main(*refs, sem), pltpu.SemaphoreType.DMA((11,)))
    pltpu.make_async_copy(refs[13], refs[13], refs[-1]).wait()


@jax.jit
def pallas_sequential_preLN__ssm_conv_s4__moe_arch_mod__prompt_kernel(
    A_u: jax.Array,
    A_A_re: jax.Array,
    A_A_im: jax.Array,
    A_B_re: jax.Array,
    A_B_im: jax.Array,
    A_C_re: jax.Array,
    A_C_im: jax.Array,
    A_log_dt: jax.Array,
    A_Dskip: jax.Array,
    B_x: jax.Array,
    B_w_r: jax.Array,
    B_w_gate: jax.Array,
    B_w_up: jax.Array,
    B_w_down: jax.Array,
):
    del B_x
    hbm = pl.BlockSpec(memory_space=pltpu.HBM)
    out = pl.pallas_call(
        _kernel,
        out_shape=jax.ShapeDtypeStruct((D, L), bf16),
        in_specs=[hbm] * 13,
        out_specs=hbm,
        scratch_shapes=[
            pltpu.VMEM((D,), bf16),
            pltpu.VMEM((D,), bf16),
            pltpu.VMEM((D,), bf16),
            pltpu.VMEM((6, D, N), bf16),
            pltpu.VMEM((3, D, 128), f32),
            pltpu.VMEM((9 * 584, N), f32),
            pltpu.VMEM((9 * 584, N), f32),
            pltpu.VMEM((6, D, N), f32),
            pltpu.VMEM((4, 5, 8, 128), f32),
            pltpu.VMEM((D, L), bf16),
            pltpu.VMEM((17 * 584, 128), f32),
            pltpu.VMEM((NT // 2, 2, 8, 256), f32),
            pltpu.VMEM((9 * 584, 128), i32),
            pltpu.VMEM((9 * 584, 128), i32),
            pltpu.VMEM((RING, 512, N), i32),
            pltpu.VMEM((RING * 8 * SS + 72, N), f32),
            pltpu.VMEM((RING, 8 * ZS + 40, N), i32),
            pltpu.VMEM((RING + 2, 8 * ZS + 40, 128), f32),
            pltpu.VMEM((RING + 2, 8, 128), i32),
            pltpu.VMEM((17 * 584, 128), f32),
            pltpu.VMEM((4, NT, 128), f32),
            pltpu.VMEM((D, L), bf16),
            pltpu.VMEM((L, 128), f32),
            pltpu.VMEM((3, DB, F), bf16),
            pltpu.VMEM((D, F), bf16),
            pltpu.VMEM((2, DB, F), bf16),
            pltpu.VMEM((DB, F), bf16),
            [pltpu.VMEM((D, 128), bf16)] * CAP,
            pltpu.SemaphoreType.DMA(()),
        ],
        compiler_params=pltpu.CompilerParams(
            vmem_limit_bytes=100 * 1024 * 1024,
            flags={"XLA_TPU_FORCE_LP_LLO_SCHEDULER": True},
        ),
    )(
        A_u.reshape(L, D).T, A_A_re, A_A_im, A_B_re, A_B_im, A_C_re, A_C_im,
        A_log_dt, A_Dskip, B_w_r, B_w_gate.reshape(3, DB, F), B_w_up,
        B_w_down.T.reshape(3, DB, F),
    )
    return out.T.reshape(1, L, D)
```

```python
import jax
import jax.numpy as jnp
from jax import lax
import jax.experimental.pallas as pl
import jax.experimental.pallas.tpu as pltpu

D = 576
L = 2048
N = 128
F = 4608
CAP = 8
EPS = 1e-5

NT = L // 128
NG = D // 8
DB = D // 3

HS = 580
PS = 577
SS = 65
ZS = 36

LAG = 8
PARTS = (LAG, 20, 40, NG)
X_ROWS = (112, 312, 488)
RING = 4
LAG_B, LAG_C, LAG_K, LAG_D = 16, 24, 42, 48
Q_LAG = 4
FW = 512
GW = 1024
NL = 13
TR = (0, 4, 12, 12, 12, 12, 12, 12, 12)
WT = {3: 5, 4: 6, 6: 7}

f32 = jnp.float32
bf16 = jnp.bfloat16
i32 = jnp.int32
NT_DIMS = (((1,), (1,)), ((), ()))


def _rnd(x):
    return x.astype(bf16).astype(f32)


def _cmul(ar, ai, br, bi):
    return ar * br - ai * bi, ar * bi + ai * br


def _csq(ar, ai):
    t = ar * ai
    return ar * ar - ai * ai, t + t


def _csqrt(wr, wi):
    big = jnp.clip(jnp.maximum(jnp.abs(wr), jnp.abs(wi)), 2.0 ** -125, 2.0 ** 125)
    e = jnp.log2(big)
    down = jnp.exp2(-e)
    xr, xi = wr * down, wi * down
    p = jnp.exp2(0.5 * jnp.log2(xr * xr + xi * xi)) + jnp.abs(xr)
    q = jnp.exp2(0.5 * ((e - 1.0) - jnp.log2(jnp.maximum(p, 2.0 ** -60))))
    t, o = p * q, xi * q
    pos = xr >= 0
    return jnp.where(pos, t, o), jnp.where(pos, o, t)


def _pack2(a, b):
    both = jnp.concatenate([a, b], axis=1).astype(bf16).reshape(2 * a.shape[0], 128)
    return pltpu.bitcast(both, i32)


def _ln_stats(s1, s2):
    m = s1 * (1.0 / D)
    v = _rnd(jnp.maximum(s2 * (1.0 / D) - m * m, 0.0))
    return _rnd(m), 1.0 / _rnd(jnp.sqrt(_rnd(v + _rnd(jnp.full_like(v, EPS)))))


def _merge(a, b):
    v = a + b[::-1]
    if len(v) > CAP:
        v = [jnp.maximum(p, q) for p, q in zip(v[:CAP], v[CAP:])]
    n = len(v) // 2
    while n:
        v = [jnp.minimum(p, v[i - n]) if i & n else jnp.maximum(p, v[i + n])
             for i, p in enumerate(v)]
        n //= 2
    return v


def _merge_rows(v):
    for n in (4, 2, 1):
        v = _merge(v, [pltpu.roll(p, n, 0) for p in v])
    return v


def _span(start, size, align):
    return pl.ds(start if isinstance(start, int) else pl.multiple_of(start, align), size)


def _lanes(c, n=1):
    return _span(128 * n * c, 128 * n, 128 * n)


def _row(ref, k, r, rows):
    return jnp.broadcast_to(ref[k, pl.ds(r, 1), :], (rows, 128))


def _iota(shape, axis):
    return lax.broadcasted_iota(i32, shape, axis)


def _lane_sum(v):
    return jnp.broadcast_to(jnp.sum(v, axis=1, keepdims=True), v.shape)


def _main(
    x_hbm, are_hbm, aim_hbm, bre_hbm, bim_hbm, cre_hbm, cim_hbm,
    ldt_hbm, dsk_hbm, wr_hbm, wg_hbm, wu_hbm, wd_hbm,
    o_hbm,
    ldt, dsk, wrt, prm, col, pr, pi, mul, vec, xb, xs, st1, un, ur,
    vs, ss, zs, ys, rs, hs, st2, nb, wg, wu, wd, we, lb, ob,
    sem_o, sem,
):
    x_mid, x_top, x_end = [(x_hbm, xb, k) for k in (4, 5, 6)]
    gate, up, down, last = (wg_hbm, wg, 7), (wu_hbm, wu, 8), (wd_hbm, wd, 9), (wd_hbm.at[2], we, 10)

    def copy(what, *where):
        src, dst, k = what
        return pltpu.make_async_copy(src.at[where], dst.at[where], sem.at[k])

    def fetch(what, after, i, c0, width, *band):
        rows = _span(8 * i, 8, 8)
        what[1][(*band, rows, _span(c0, 128, 128))] = after.astype(bf16)
        copy(what, *band, rows, _span(c0, width, 128)).start()

    def queue(what, m):
        bands, c0 = (4, GW) if what is gate else (2, 0)
        width = (F - c0) // 4
        copy(what, slice(0, bands), _span(8 * (m >> 2), 8, 8),
             _span(c0 + width * (m & 3), width, 128)).start(priority=1)

    v_cp = [pltpu.make_async_copy(a, b, sem.at[0])
            for a, b in ((ldt_hbm, ldt), (dsk_hbm, dsk), (wr_hbm, wrt))]
    p_cp = {0: [copy((src, prm.at[k], 11), slice(0, 8 * PARTS[0]))
                for k, src in enumerate((are_hbm, aim_hbm))]}
    p_cp |= {lo: [copy((src, prm.at[k], 1 + j), slice(8 * (lo - LAG * (k > 1)),
                                                       8 * (hi - LAG * (k > 1 and hi < NG))))
                  for k, src in enumerate((are_hbm, aim_hbm, bre_hbm, bim_hbm, cre_hbm, cim_hbm))]
             for j, (lo, hi) in enumerate(zip(PARTS, PARTS[1:]))}
    x0, x1, x2 = X_ROWS
    held_back = []
    for k, c in enumerate(sum(p_cp.values(), v_cp)
                          + [copy(x_mid, slice(x0, x1)), copy(x_top, slice(0, x0))]):
        if k in (15, 16):
            held_back.append(c)
        else:
            c.start(priority=int(k > 10 or (k > 4 and k % 2)))

    lane8, sub8 = _iota((8, 128), 1), _iota((8, 128), 0)
    zero8, zero16 = jnp.zeros((8, 128), f32), jnp.zeros((16, 128), f32)
    nb[...] = jnp.zeros((L, 128), f32)
    for c in v_cp:
        c.wait()
    for c in held_back:
        c.start()
    for k, ref in enumerate((ldt, dsk, wrt)):
        row = ref[...].astype(f32).reshape(1, D)
        row = jnp.concatenate([row, jnp.zeros((1, 640 - D), f32)], axis=1)
        for t in range(5):
            v = jnp.broadcast_to(row[:, 128 * t:128 * t + 128], (8, 128))
            vec[k, t] = v if k else _rnd(jnp.exp(v))

    def own(k, g):
        return jnp.where(lane8 - sub8 == 8 * (g & 15), vec[k, g >> 4], 0.0)

    def step_size(g):
        col[2, _span(8 * g, 8, 8), :] = _lane_sum(own(0, g))

    paced = (D - x1) // 4
    pl.loop(0, NG - paced, unroll=NG - paced)(step_size)
    vec[3, 0] = _lane_sum(sum(vec[2, t] for t in range(5)))

    zero = jnp.minimum(pltpu.bitcast(vec[1, 0], i32)[0, 0] & 1, 0)
    never = (lane8 < zero, sub8 < zero)

    def step(g, *after):
        rows = _span(8 * g, 8, 8)
        dt = col[2, rows, :]
        for mask, v in zip(never, after):
            dt = jnp.where(mask, v, dt)
        mag, ph = jnp.exp(dt * prm[0, rows, :].astype(f32)), dt * prm[1, rows, :].astype(f32)
        cos = jnp.cos(ph)
        mul[4, rows, :], mul[5, rows, :] = mag * cos, mag * jnp.sin(ph)
        return mag, cos

    def powers(g, after):
        rows = _span(8 * g, 8, 8)
        dt = jnp.where(never[0], after, col[2, rows, :])
        br, bi, cr, ci = [prm[k, rows, :].astype(f32) for k in range(2, 6)]
        w = _cmul(cr, ci, dt * br, dt * bi)
        col[0, rows, :] = _lane_sum(w[0] + own(1, g))
        col[1, rows, :] = _lane_sum(own(2, g))
        a = mul[4, rows, :], mul[5, rows, :]
        v = _csqrt(*_cmul(*w, *a))
        a = _csq(*a)
        for j in range(8):
            pr[pl.ds(j * PS + rows.start, 8), :], pi[pl.ds(j * PS + rows.start, 8), :] = v
            done, v = v[0], _cmul(*v, *a)
        for _ in range(3):
            a = _csq(*a)
        mul[0, rows, :], mul[1, rows, :] = a
        mul[2, rows, :], mul[3, rows, :] = _csq(*_csq(*a))
        return done

    def set_up(lo, hi, carry):
        def one(g, carry):
            trig, done = carry
            mag = cos = new = trig[0]
            if lo < NG:
                mag, cos = step(g, trig[0], done[0])
            if lo < paced:
                step_size(g + NG - paced)
                fetch(x_mid if 4 * lo < x2 - x1 else x_end, mag,
                      x1 // 8 + (g >> 1), L // 2 * (g & 1), L // 2)
            if lo >= LAG:
                new = powers(g - LAG, trig[0])
            return trig[1:] + [cos], done[1:] + [new]

        return lax.fori_loop(lo, hi, one, carry, unroll=hi - lo)

    carry = ([zero8] * 3, [zero8] * 4)
    cuts = sorted(PARTS + (0, (x2 - x1) // 4, paced, NG + LAG))
    for lo, hi in zip(cuts, cuts[1:]):
        for c in p_cp.get(lo, []):
            c.wait()
        for m in range(18 if lo == PARTS[-2] else 0):
            queue(gate, m)
        carry = set_up(lo, hi, carry)

    def moments(i, part, rows, after):
        s1 = s2 = jnp.concatenate([jnp.where(never[0], after, 0.0)] * 2, axis=1)
        if part:
            s1, s2 = st1[i, 0], st1[i, 1]
        for q in rows:
            v = xb[pl.ds(q, 8), _lanes(i, 2)].astype(f32)
            for e in range(2):
                xs[pl.ds((2 * i + e) * HS + q, 8), :] = v[:, 128 * e:128 * e + 128]
            s1, s2 = s1 + v, s2 + v * v
            if q == 0:
                fetch(down, s1[:, :128], i >> 1, F // 3 * 2, F // 3, i & 1)
        fetch(down, v[:, :128], i >> 1, F // 3 * part, F // 3, i & 1)
        if part:
            s1, s2 = _ln_stats(*[jnp.broadcast_to(jnp.sum(v, axis=0, keepdims=True), v.shape)
                                 for v in (s1, s2)])
        st1[i, 0], st1[i, 1] = s1, s2
        return s2[:, :128]

    flip = jnp.where(_iota((128, 128), 0) == _iota((128, 128), 1) ^ 63, 1.0, 0.0).astype(bf16)

    def normalise(i):
        m, s = [[st1[i, n, :, _lanes(e)] for e in range(2)] for n in range(2)]
        for q in range(D // 16):
            xa, xc = [[xs[pl.ds(c * HS + 16 * q + 8 * e, 8), :] for e in range(2)]
                      for c in (2 * i, 2 * i + 1)]
            u = [((xa[e] - m[0]) * s[0], (xc[e] - m[1]) * s[1]) for e in range(2)]
            w = [_pack2(*v) for v in u]
            if q % 3 == 0:
                r = jnp.dot(jnp.concatenate(u[0] + u[1], axis=0).astype(bf16), flip,
                            preferred_element_type=f32)
                r = [_pack2(r[n:n + 8], r[n + 8:n + 16]) for n in (0, 16)]
            else:
                r = [jnp.take_along_axis(v, lane8 ^ 63, axis=1, mode="promise_in_bounds")
                     for v in w]
            for e in range(2):
                rows = pl.ds(i * HS + 16 * q + 8 * e, 8)
                un[rows, :], ur[rows, :] = w[e], r[e]


    @pl.loop(0, 1 + zero)
    def _(_):
        for part, spans in enumerate(([(x_mid, x0, x2)], [(x_top, 0, x0), (x_end, x2, D)])):
            for what, a, b in spans:
                copy(what, slice(a, b)).wait()
            rows = [q for _, a, b in spans for q in range(a, b, 8)]
            lax.fori_loop(0, NT // 2, lambda i, v: moments(i, part, rows, v), zero8,
                          unroll=NT // 2)
        pl.loop(0, NT // 2, unroll=NT // 2)(normalise)

    left8, right8 = lane8 < 64, lane8 >= 64
    lane16, row16 = _iota((16, 128), 1), _iota((16, 128), 0)
    lane32, row32 = _iota((32, 128), 1), 2 * _iota((32, 128), 0)
    tri0, tri1 = (lane32 >= row32) & (lane32 < 64), lane32 >= row32 + 64

    def v_tile(r, k):
        return pltpu.bitcast(vs[r, pl.ds(64 * k, 64), :], bf16)

    def channel(ref, g, k, n):
        return ref[pl.ds(g * 8 + k, n, stride=HS), :]

    def vandermonde(g, r, k):
        ch = g * 8 + k
        vr, vi = pr[pl.ds(ch, 8, stride=PS), :], pi[pl.ds(ch, 8, stride=PS), :]
        odd = _cmul(vr, vi, _row(mul, 4, ch, 8), _row(mul, 5, ch, 8))
        vr, vi = jnp.concatenate([vr, odd[0]], axis=0), jnp.concatenate([vi, odd[1]], axis=0)
        mr, mi = _row(mul, 0, ch, 16), _row(mul, 1, ch, 16)
        re, im = [], []
        for q in range(4):
            re.append(_pack2(vr[:8], vr[8:]))
            im.append(_pack2(vi[:8], vi[8:]))
            vr, vi = _cmul(vr, vi, mr, mi)
        for q, v in enumerate(re + im):
            vs[r, pl.ds(64 * k + 8 * q, 8), :] = v
        return odd[0]

    def chunk_states(g, r, k):
        p1 = channel(ur, g, k, NT // 2)
        p2 = pltpu.roll(p1, 64, 1)
        lhs = jnp.concatenate([
            jnp.where(left8, p1, 0), jnp.where(right8, p2, 0),
            jnp.where(left8, p2, 0), jnp.where(right8, p1, 0)], axis=0)
        ss[pl.ds(SS * (8 * r + k), 64), :] = jnp.dot(
            pltpu.bitcast(lhs, bf16), v_tile(r, k), preferred_element_type=f32)

    def scan(g, r, k, state):
        def s_at(row):
            return ss[pl.ds(SS * 8 * r + row, 8, stride=SS), :]

        seen = []
        if k == 0:
            rows = _span(8 * g, 8, 8)
            seen.append((pr[rows, :], -pi[rows, :]))
            state = (mul[2, rows, :], mul[3, rows, :], s_at(0), -s_at(16))
        cr, ci, xr, xi = state
        for h in range(max(4 * k, 1), 4 * k + 4):
            seen.append((xr, xi))
            base = 32 * (h % 2) + h // 2
            if h < 31:
                xr, xi = ((cr * xr + s_at(base)) + ci * xi,
                          (cr * xi - s_at(base + 16)) - ci * xr)
        for e in range(2):
            for p in range(2):
                zs[r, pl.ds(16 * e + 8 * p + k, 8, stride=ZS), :] = _pack2(
                    seen[e][p], seen[2 + e][p])
        return cr, ci, xr, xi

    def read_out(r, k, y):
        o = lax.dot_general(pltpu.bitcast(zs[r, pl.ds(ZS * k, 32), :], bf16), v_tile(r, k),
                            NT_DIMS, preferred_element_type=f32)
        ys[y, pl.ds(ZS * k, 16), :] = jnp.where(lane16 < 64, o[0:16], o[48:64])
        ys[y, pl.ds(ZS * k + 16, 16), :] = jnp.where(lane16 < 64, o[32:48], o[16:32])

    def taps(g, r):
        ra, rb = pl.ds(0, 8, stride=ZS), pl.ds(16, 8, stride=ZS)
        ya, yb = ys[r, ra, :], ys[r, rb, :]
        ys[r, ra, :], ys[r, rb, :] = jnp.where(left8, 0.0, ya), jnp.where(left8, yb, 0.0)
        kk = jnp.where(left8, ya, yb)
        diag = col[0, _span(8 * g, 8, 8), :]
        ka = pltpu.roll(kk, 1, 1) + pltpu.roll(kk, 65, 1)
        kb = pltpu.roll(kk, 2, 1) + pltpu.roll(kk, 66, 1)
        pos = lane8 & 63
        rs[r] = _pack2(jnp.where(pos == 0, diag, ka),
                       jnp.where(pos == 0, 0.0, jnp.where(pos == 1, diag, kb)))

    def finish(g, r, k, older, acc):
        yq = pltpu.roll(ys[r, pl.ds(ZS * k + 16, 16), :], 64, 1)
        rb = pltpu.roll(_row(rs, r, k, 32), 0, 1, stride=2, stride_axis=0)
        t = jnp.concatenate([jnp.where(tri0, rb, 0), jnp.where(tri1, rb, 0)], axis=0)
        u = channel(un, g, k, NT // 2)
        for e in range(0 if older is None else 2):
            u = jnp.where(never[e], pltpu.bitcast(older[8 * e:8 * e + 8], i32), u)
        y = jnp.dot(pltpu.bitcast(u, bf16), pltpu.bitcast(t, bf16), preferred_element_type=f32)
        h = y + (channel(xs, g, k, NT) + (yq + ys[r, pl.ds(ZS * k, 16), :]))
        hs[pl.ds(g * 8 + k, NT, stride=HS), :] = h
        return yq, h[:8], (acc[0] + h, acc[1] + h * h, acc[2] + h * _row(col, 1, g * 8 + k, NT))

    def pace(g, k, after):
        if k == 7:
            fetch(gate, after, g >> 2, 0, GW, g & 3)
        elif k % 2:
            q, r = (3 * g + k // 2) >> 2, (3 * g + k // 2) & 3
            fetch(up, after, r * (NG // 4) + lax.div(q, 3), F // 3 * lax.rem(q, 3), F // 3)

    def body(what, g0, q0, steps, carry):
        acc, rolled = carry[0], dict(zip(range(-Q_LAG, 0), carry[1]))
        state = None
        for t in range(steps):
            def at(lag):
                q, k = divmod(t - lag, 8)
                if q0 + q >= 0:
                    return g0 + q, (q0 + q) % RING, k

            if w := at(LAG_C):
                read_out(*w[1:], w[1])
            pace(g0 + t // 8, t % 8, vandermonde(*at(0)))
            if t % 4 == 0 and what is down:
                queue(down, 24 - NG + 2 * g0 + t // 4)
            elif t % 4 == 0 and t % 16 < 12:
                queue(gate, 18 + 3 * (g0 >> 1) + t // 4 - t // 16)
            if w := at(LAG_B):
                state = scan(*w, state)
            chunk_states(*at(0))
            if (w := at(LAG_K)) and w[2] == 0:
                taps(*w[:2])
            if w := at(LAG_D):
                rolled[t], _, acc = finish(*w, rolled.get(t - Q_LAG), acc)
        return acc, [rolled[t] for t in range(steps - Q_LAG, steps)]

    fill, n = pl.cdiv(LAG_D + Q_LAG, 8 * RING), NG // RING

    def steady(what, lo, hi, carry):
        return lax.fori_loop(lo, hi, lambda j, c: body(what, j * RING, fill * RING, 8 * RING, c),
                             carry, unroll=hi - lo)[0]

    spare = list(range(3 * NL))

    def fetch_last(after):
        r, c = divmod(spare.pop(), 3)
        fetch(last, after, DB // 8 - NL + r, F // 3 * c, F // 3)

    def first_half(acc):
        return steady(gate, fill, n // 2, body(gate, 0, 0, 8 * RING * fill, (acc, [])))

    def second_half(acc):
        for m in range(16, 24):
            queue(down, m)
        return steady(down, n // 2, n, (acc, [zero16] * Q_LAG))

    def drain(acc):
        def slot(g):
            return g % RING + 2 * (g >= NG - 2)

        copy(last, slice(0, DB - 8 * NL)).start(priority=1)
        state = None
        for ch in range(D - LAG_B, D):
            state = scan(ch // 8, ch // 8 % RING, ch % 8, state)
            if ch < D - 8 and ch % 2 == 0:
                fetch_last(state[2])
        for g in (NG - 5, NG - 4):
            taps(g, slot(g))
        for ch in range(D - LAG_C, D):
            read_out(ch // 8 % RING, ch % 8, slot(ch // 8))
            if ch % 4 == 0 and ch > D - LAG_C:
                fetch_last(ys[slot(ch // 8), pl.ds(ZS * (ch % 8), 8), :])
        for ch in range(D - LAG_D, D):
            for g in range(NG - 3, NG if ch == D - 32 else 0):
                taps(g, slot(g))
            g, k = divmod(ch, 8)
            _, h, acc = finish(g, slot(g), k, None, acc)
            if ch % 6 == 5:
                fetch_last(h)
        return acc

    acc = (zero16,) * 3
    for part in (first_half, second_half, drain):
        acc = lax.fori_loop(0, 1 + zero, lambda _, c: part(c), acc)

    m2, inv2 = _ln_stats(acc[0], acc[1])
    score = (acc[2] - m2 * jnp.concatenate([vec[3, 0]] * 2)) * inv2
    st2[0], st2[1], st2[2] = m2, inv2, _rnd(score)

    bits = pltpu.bitcast(jnp.where(score == 0.0, 0.0, score), i32) >> 13
    rank = jnp.where(score != score, 0, jnp.where(bits >= 0, bits + (1 << 18), -1 - bits))
    key = pltpu.bitcast((1 << 29) + (rank << 11) + (L - 1 - (row16 * 128 + lane16)), f32)

    def write_tiles(j, after, run):
        m, s = [[_row(st2, n, 2 * j + e, 8) for e in range(2)] for n in range(2)]
        scale, shift = [v + 1.0 for v in s], [a * b for a, b in zip(m, s)]

        def some(i, done):
            mult = [jnp.where(never[0], done[0], v) for v in scale]
            for q in range(run):
                rows = _span(8 * (run * i + q), 8, 8)
                v = [hs[pl.ds((2 * j + e) * HS + rows.start, 8), :] * mult[e] - shift[e]
                     for e in range(2)]
                ob[rows, _lanes(j, 2)] = jnp.concatenate(v, axis=1).astype(bf16)
            return done[1], v[1]

        done = after, after
        for lo, hi in ((0, 12), (12, 48), (48, NG)):
            if lo and j < 5:
                fetch_last(done[1])
            done = lax.fori_loop(lo // run, hi // run, some, done, unroll=(hi - lo) // run)
        return done[1]

    def spread(v, shift, stride, after):
        return [jnp.where(never[1], after, pltpu.roll(p, shift, 1, stride=stride, stride_axis=0))
                for p in v]

    tops = _merge_rows(_merge([key[:8]], [key[8:]]))
    tops = _merge_rows(spread(tops, 0, 1, write_tiles(0, tops[0], 3)))
    after = write_tiles(1, tops[0], 3)
    tops = _merge_rows(_merge(spread(tops, 0, 8, after), spread(tops, 64, 8, after)))
    after = tops[0]
    for j in (2, 3, 4):
        after = write_tiles(j, after, 2)
    st2[3] = jnp.where(key >= jnp.concatenate([tops[-1]] * 2), 1.0, 0.0)
    tops = [~pltpu.bitcast(v, i32) & (L - 1) for v in tops]
    tops = [[pltpu.bitcast((1 << 29) + ((v & 127) << 11) + v, f32)] for v in tops]
    while len(tops) > 1:
        tops = [_merge(a, b) for a, b in zip(tops[::2], tops[1::2])]
    idx = [pltpu.bitcast(v, i32)[0, 0] & (L - 1) for v in tops[0]]

    tile, lane = [v >> 7 for v in idx], [v & 127 for v in idx]
    turn, turns = [0, 0], 0
    for j in range(2, CAP):
        turn.append(jnp.where(lane[j] == lane[j - 2], turn[j - 2] + 1, 0))
        turns = jnp.maximum(turns, turn[j] + 1)

    def gather(n):
        at = [jnp.where(turn[j] == n, lane[j], -1) for j in range(CAP)]
        rows = []
        for team in (range(0, CAP, 2), range(1, CAP, 2)):
            onehot, merged = zero8, []
            for j in team:
                onehot = jnp.where((sub8 == j) & (lane8 == at[j]), 1.0, onehot)
            for q in range(0, D, 16):
                v = hs[pl.ds(tile[team[0]] * HS + q, 16), :]
                for j in team[1:]:
                    v = jnp.where(lane16 == at[j], hs[pl.ds(tile[j] * HS + q, 16), :], v)
                merged.append(v)
            merged = jnp.concatenate(merged + merged[-4:], axis=0).astype(bf16)
            rows.append(lax.dot_general(onehot.astype(bf16), merged, NT_DIMS,
                                        preferred_element_type=f32))
        stat = [zero8] * 3
        for j in range(CAP):
            pick = (sub8 == j) & (lane8 == at[j])
            stat = [jnp.where(pick, _row(st2, k, tile[j], 8), v) for k, v in enumerate(stat)]
        return [rows[0] + rows[1]] + [_lane_sum(v) for v in stat]

    hsel, m_j, s_j, r_j = lax.fori_loop(
        1, turns, lambda n, c: [a + b for a, b in zip(c, gather(n))], gather(0))
    xsel = _rnd(_rnd(hsel - jnp.tile(m_j, (1, 5))) * jnp.tile(s_j, (1, 5)))

    x_main = xsel[:, :512].astype(bf16)
    x_tail = jnp.concatenate([xsel[:, 512:]] * 2, axis=0)
    x_tail = jnp.where((row16 < 8) == (lane16 < 64), x_tail, 0.0).astype(bf16)
    for v in (m_j, xsel[:, :128]):
        fetch_last(v)
    for c in (copy(gate, slice(None)), copy(up, slice(None)), copy(down, slice(0, 2))):
        c.wait()
    for v in (m_j, m_j):
        fetch_last(v)

    late, fresh = 0, []
    for j in range(CAP):
        fresh.append(((late >> tile[j]) & 1) == 0)
        late = late | (1 << tile[j])

    def bands(ref, cols):
        v = ref[:, :, cols]
        return v.reshape(-1, v.shape[2])

    acts, w_t = [], []

    def transpose_ahead(v):
        b, t = divmod(len(w_t), F // 128)
        if b == 3:
            return v
        w_t.append(pltpu.bitcast(bands(wd, _lanes(t))[128 * b:128 * b + 128].T, i32))
        if t % 3 == 0 and spare:
            fetch_last(pltpu.bitcast(w_t[-1][:8], f32))
        return jnp.where(never[t % 2], pltpu.bitcast(w_t[-1][56:], v.dtype) + v, v)

    popped, sent = [xsel[:, :128]] * 2, 0
    for k in range(F // FW):
        f = pl.ds(k * FW, FW)
        x_k = pltpu.bitcast(x_tail, i32)
        for _ in range(TR[k]):
            x_k = transpose_ahead(x_k)
        if k in WT:
            x_k = jnp.where(never[1], pltpu.bitcast(write_tiles(WT[k], popped[-2], 1), i32), x_k)
            for c in range(sent, sent := 2 * WT[k] + 2):
                pl.when(((late >> c) & 1) == 0)(lambda: pltpu.make_async_copy(
                    ob.at[:, _lanes(c)], o_hbm.at[:, _lanes(c)], sem_o).start(priority=c % 2))
        tail = jnp.concatenate([bands(wg, f)[512:], wu[pl.ds(512, 64), f]], axis=0)
        tail = jnp.dot(pltpu.bitcast(x_k, bf16), tail, preferred_element_type=f32)
        a = jnp.dot(x_main, bands(wg, f)[:512], preferred_element_type=f32)
        b = jnp.dot(x_main, wu[pl.ds(0, 512), f], preferred_element_type=f32)
        popped.append(b[:8, :128])
        a, b = _rnd(a + tail[:8]), _rnd(b + tail[8:])
        act = _rnd(a * jax.nn.sigmoid(a)) * b
        acts += [act[:, n:n + 128] for n in range(0, FW, 128)]
    weight = _rnd(jax.nn.sigmoid(r_j))
    routed = [_row(st2, 3, v, 8) > 0 for v in tile]

    def project(d0, ties):
        nd = min(128, D - d0)
        y = jnp.zeros((8, nd), f32)
        for t, act in enumerate(acts):
            if d0 or t >= 12:
                act = transpose_ahead(act)
            if t in ties:
                act = jnp.where(never[0], ties[t], act)
            if d0 < 2 * DB:
                y = y + jnp.dot(act.astype(bf16), pltpu.bitcast(w_t[d0 // 128 * len(acts) + t], bf16),
                                preferred_element_type=f32)
            else:
                y = y + lax.dot_general(act.astype(bf16), we[pl.ds(d0 - 2 * DB, nd), _lanes(t)],
                                        NT_DIMS, preferred_element_type=f32)
        return y

    def patch(d0, y):
        nd = y.shape[1]
        rows = pl.ds(d0, nd)
        new = hsel[:, d0:d0 + nd] + _rnd(xsel[:, d0:d0 + nd] + _rnd(_rnd(y) * weight[:, :nd]))
        if nd < 128:
            new = jnp.concatenate([new, zero8[:, nd:]], axis=1)
        for j in range(CAP):
            nb[pl.ds(idx[j], 1), :] = new[j:j + 1]
        for j in range(CAP):
            cols = _lanes(tile[j])
            one = pltpu.bitcast(nb[cols, :].astype(bf16).T[:nd], i32)
            for q in range(0, nd, 16):
                lb[j][pl.ds(d0 + q, 16), :] = pltpu.bitcast(jnp.where(
                    routed[j], one[q // 2:q // 2 + 8],
                    pltpu.bitcast(ob[pl.ds(d0 + q, 16), cols], i32)), bf16)
        for j in range(CAP):
            pl.when(fresh[j])(lambda: pltpu.make_async_copy(
                lb[j].at[rows], o_hbm.at[rows, _lanes(tile[j])], sem_o).start(priority=j % 2))
        return new, pltpu.bitcast(one[-8:], f32)

    begun, ended = patch(0, project(0, {}))
    held = project(128, {19: begun}), project(256, {32: ended})
    assert not spare
    copy(last, slice(None)).wait()
    ended = patch(128, held[0])[1], patch(256, held[1])[1]
    begun = patch(384, project(384, dict(zip((28, 35), ended))))[0]
    patch(512, project(512, {19: begun}))


def _kernel(*refs):
    pl.run_scoped(lambda sem: _main(*refs, sem), pltpu.SemaphoreType.DMA((12,)))
    o_hbm, ob, sem_o = refs[13], refs[-2], refs[-1]
    pltpu.make_async_copy(ob, o_hbm, sem_o).wait()


@jax.jit
def pallas_sequential_preLN__ssm_conv_s4__moe_arch_mod__prompt_kernel(
    A_u: jax.Array,
    A_A_re: jax.Array,
    A_A_im: jax.Array,
    A_B_re: jax.Array,
    A_B_im: jax.Array,
    A_C_re: jax.Array,
    A_C_im: jax.Array,
    A_log_dt: jax.Array,
    A_Dskip: jax.Array,
    B_x: jax.Array,
    B_w_r: jax.Array,
    B_w_gate: jax.Array,
    B_w_up: jax.Array,
    B_w_down: jax.Array,
):
    del B_x
    hbm = pl.BlockSpec(memory_space=pltpu.HBM)
    out = pl.pallas_call(
        _kernel,
        out_shape=jax.ShapeDtypeStruct((D, L), bf16),
        in_specs=[hbm] * 13,
        out_specs=hbm,
        scratch_shapes=[
            pltpu.VMEM((D,), bf16),
            pltpu.VMEM((D,), bf16),
            pltpu.VMEM((D,), bf16),
            pltpu.VMEM((6, D, N), bf16),
            pltpu.VMEM((3, D, 128), f32),
            pltpu.VMEM((9 * 584, N), f32),
            pltpu.VMEM((9 * 584, N), f32),
            pltpu.VMEM((6, D, N), f32),
            pltpu.VMEM((4, 5, 8, 128), f32),
            pltpu.VMEM((D, L), bf16),
            pltpu.VMEM((17 * 584, 128), f32),
            pltpu.VMEM((NT // 2, 2, 8, 256), f32),
            pltpu.VMEM((9 * 584, 128), i32),
            pltpu.VMEM((9 * 584, 128), i32),
            pltpu.VMEM((RING, 512, N), i32),
            pltpu.VMEM((RING * 8 * SS + 72, N), f32),
            pltpu.VMEM((RING, 8 * ZS + 40, N), i32),
            pltpu.VMEM((RING + 2, 8 * ZS + 40, 128), f32),
            pltpu.VMEM((RING + 2, 8, 128), i32),
            pltpu.VMEM((17 * 584, 128), f32),
            pltpu.VMEM((4, NT, 128), f32),
            pltpu.VMEM((L, 128), f32),
            pltpu.VMEM((4, D // 4, F), bf16),
            pltpu.VMEM((D, F), bf16),
            pltpu.VMEM((2, DB, F), bf16),
            pltpu.VMEM((DB, F), bf16),
            [pltpu.VMEM((D, 128), bf16)] * CAP,
            pltpu.VMEM((D, L), bf16),
            pltpu.SemaphoreType.DMA(()),
        ],
        compiler_params=pltpu.CompilerParams(
            vmem_limit_bytes=100 * 1024 * 1024,
            flags={"XLA_TPU_FORCE_LP_LLO_SCHEDULER": True},
        ),
    )(
        A_u.reshape(L, D).T, A_A_re, A_A_im, A_B_re, A_B_im, A_C_re, A_C_im,
        A_log_dt, A_Dskip, B_w_r, B_w_gate.reshape(4, D // 4, F), B_w_up,
        B_w_down.T.reshape(3, DB, F),
    )
    return out.T.reshape(1, L, D)
```
